```python
import jax
import jax.numpy as jnp

def _softmax(x, axis=-1):
    return jax.nn.softmax(x, axis=axis)

def _gelu(x):
    return jax.nn.gelu(x, approximate=True)

def _silu(x):
    return jax.nn.silu(x)

def _sigmoid(x):
    return jax.nn.sigmoid(x)

def _layernorm(x, axis=-1, eps=1e-05):
    m = jnp.mean(x, axis=axis, keepdims=True)
    v = jnp.var(x, axis=axis, keepdims=True)
    return (x - m) / jnp.sqrt(v + eps)

def _scatter_add(tgt, idx, src, axis=0):
    return tgt.at[idx].add(src)

def _segment_sum(src, seg, n):
    return jax.ops.segment_sum(src, seg, n)

class _Rng:

    def __init__(self, key):
        self._k = key

    def _next(self):
        self._k, sub = jax.random.split(self._k)
        return sub

    def normal(self, shape):
        return jax.random.normal(self._next(), shape, dtype=jnp.bfloat16)

    def randint(self, lo, hi, shape):
        return jax.random.randint(self._next(), shape, lo, hi, dtype=jnp.int32)

    def uniform(self, shape, lo=0.0, hi=1.0):
        return jax.random.uniform(self._next(), shape, jnp.bfloat16, lo, hi)

    def permutation(self, n):
        return jax.random.permutation(self._next(), n)
kernel_name = 'adaLN_cond__sliding_block_cached__moe_arch_mod__prompt'

def setup_inputs():
    _rng = _Rng(jax.random.key(int.from_bytes(__import__("os").urandom(4), "little")))
    _w = lambda a: (lambda t: t.astype(jnp.bfloat16) if jnp.issubdtype(t.dtype, jnp.floating) else t)(jnp.asarray(a))

    def _A_setup():
        B, Sq, D = (1, 2048, 1024)
        Hq, Hkv, Sk, Dh = (32, 4, 2048, 128)
        assert Hq % Hkv == 0, (Hq, Hkv)
        return {'x': _w((lambda *s: _rng.normal(s) * 0.05)(B, Sq, D)), 'k_cache': _w((lambda *s: _rng.normal(s) * 0.05)(B, Hkv, Sk, Dh)), 'v_cache': _w((lambda *s: _rng.normal(s) * 0.05)(B, Hkv, Sk, Dh)), 'wq': _w((lambda *s: _rng.normal(s) * 0.05)(D, Hq * Dh) * D ** (-0.5)), 'wo': _w((lambda *s: _rng.normal(s) * 0.05)(Hq * Dh, D) * (Hq * Dh) ** (-0.5))}
    _A_in = _A_setup()

    def _B_setup():
        B, S, D, F, C = (1, 2048, 1024, 3584, 1)
        return {'x': _w((lambda *s: _rng.normal(s) * 0.05)(B, S, D)), 'w_r': _w((lambda *s: _rng.normal(s) * 0.05)(D)), 'w_gate': _w((lambda *s: _rng.normal(s) * 0.05)(D, F)), 'w_up': _w((lambda *s: _rng.normal(s) * 0.05)(D, F)), 'w_down': _w((lambda *s: _rng.normal(s) * 0.05)(F, D))}
    _B_in = _B_setup()
    return {'A_x': _A_in['x'], 'A_k_cache': _A_in['k_cache'], 'A_v_cache': _A_in['v_cache'], 'A_wq': _A_in['wq'], 'A_wo': _A_in['wo'], 'B_x': _B_in['x'], 'B_w_r': _B_in['w_r'], 'B_w_gate': _B_in['w_gate'], 'B_w_up': _B_in['w_up'], 'B_w_down': _B_in['w_down'], 'c': _w((lambda *s: _rng.normal(s) * 0.05)(1, 1024)), 'w_mod': _w((lambda *s: _rng.normal(s) * 0.05)(1024, 6 * 1024) * 1024 ** (-0.5))}

def reference(A_x, A_k_cache, A_v_cache, A_wq, A_wo, B_x, B_w_r, B_w_gate, B_w_up, B_w_down, c, w_mod):

    def _A_ref(x, k_cache, v_cache, wq, wo):
        B, Sq, D = x.shape
        Hq, Dh = (32, 128)
        Hkv, Sk = (k_cache.shape[1], k_cache.shape[2])
        W = min(4096, max(256, Sk // 4))
        rep = Hq // Hkv
        q = (lambda x, *d: x.transpose(*d))((x @ wq).reshape(B, Sq, Hq, Dh), 0, 2, 1, 3)
        k = jnp.repeat(k_cache[:, :, Sk - W:, :], rep, axis=1)
        v = jnp.repeat(v_cache[:, :, Sk - W:, :], rep, axis=1)
        scores = jnp.einsum('bhqd,bhkd->bhqk', q, k) * Dh ** (-0.5)
        p = _softmax(scores, axis=-1)
        o = jnp.einsum('bhqk,bhkd->bhqd', p, v)
        return (lambda x, *d: x.transpose(*d))(o, 0, 2, 1, 3).reshape(B, Sq, Hq * Dh) @ wo

    def _B_ref(x, w_r, w_gate, w_up, w_down):
        B, S, D = x.shape
        C = 1
        r = x @ w_r
        idx = jnp.argsort(-r, axis=-1)[:, :C]
        idx_e = jnp.repeat(idx.reshape(B, C, 1), D, axis=2)
        x_sel = jnp.take_along_axis(x, idx_e, axis=1)
        g = _silu(x_sel @ w_gate)
        u = x_sel @ w_up
        y = g * u @ w_down
        r_sel = _sigmoid(jnp.take_along_axis(r, idx, axis=1))
        y = y * r_sel.reshape(B, C, 1)
        b_off = (jnp.arange(B) * S).reshape(B, 1)
        flat_idx = (idx + b_off).reshape(B * C)
        zero = (x * 0.0).reshape(B * S, D)
        upd = _scatter_add(zero, flat_idx, y.reshape(B * C, D), axis=0)
        return x + upd.reshape(B, S, D)
    x = A_x
    mod = (_silu(c) @ w_mod).reshape(c.shape[0], 6, 1, -1)
    sa, ca, ga, sb, cb, gb = (mod[:, 0].copy(), mod[:, 1].copy(), mod[:, 2].copy(), mod[:, 3].copy(), mod[:, 4].copy(), mod[:, 5].copy())
    h = _layernorm(x, axis=-1) * (1 + ca) + sa
    x = x + ga * _A_ref(h, A_k_cache, A_v_cache, A_wq, A_wo)
    h = _layernorm(x, axis=-1) * (1 + cb) + sb
    x = x + gb * _B_ref(h, B_w_r, B_w_gate, B_w_up, B_w_down)
    return x
```

```python
import functools
import jax
import jax.numpy as jnp
import numpy as np
from jax import lax
import jax.experimental.pallas as pl
import jax.experimental.pallas.tpu as pltpu

S, D = 2048, 1024
HQ, HKV, DH = 32, 4, 128
SK = 2048
W = 512
REP = HQ // HKV
F = 3584
EPS = 1e-5
LOG2E = 1.4426950408889634
BM = 256
NB = S // BM
NT = D // 128
NF = F // 128
NMOD = 6 * NT
SUB = 16
HM = BM // 2
KH = HQ * DH // 2
NH = NT // 2
HH = HQ // 2

f32 = jnp.float32
bf16 = jnp.bfloat16
u32 = jnp.uint32
NT_DIMS = (((1,), (1,)), ((), ()))


def _rows(m8, n):
    return jnp.concatenate([m8] * (n // 8), axis=0) if n > 8 else m8


def _ln_mod(x, scale1p, shift):
    m = jnp.mean(x, axis=-1, keepdims=True)
    xc = x - m
    v = jnp.mean(xc * xc, axis=-1, keepdims=True)
    return xc * lax.rsqrt(v + EPS) * scale1p + shift


def _b(u):
    return pltpu.bitcast(u, bf16)


def _u(b):
    return pltpu.bitcast(b, u32)


def kernel(x_hbm, k_hbm, v_hbm, wq_hbm, wo_hbm, wr_hbm, wg_hbm, wu_hbm, wd_hbm, c_hbm, wmod_hbm,
           out_hbm,
           xo_v, k_v, wq_v, wo_v, wr_v, wg_v, wu_v, wd_v, c_v, wmod_v,
           he_v, ho_v, o_v, qa_v, qb_v, mod_v, wbac_v, acca_v, accb_v, slab_v,
           sx, swq, swo, swm, swg, swu, swd, so, sv, sk, sm):
    x_v = xo_v.at[0]
    h2_v = xo_v.at[1]
    out_v = xo_v.at[2]
    wq_u = wq_v.bitcast(u32)
    wo_u = wo_v.bitcast(u32)
    wg_u = wg_v.bitcast(u32)
    wu_u = wu_v.bitcast(u32)
    wd_u = wd_v.bitcast(u32)
    wmod_u = wmod_v.bitcast(u32)
    he_u = he_v.bitcast(u32)
    ho_u = ho_v.bitcast(u32)
    o_u = o_v.bitcast(u32)
    qa_u = qa_v.bitcast(u32)
    qb_u = qb_v.bitcast(u32)
    k_u = k_v.bitcast(u32)
    wbac_u = wbac_v.bitcast(u32)

    cp_c = pltpu.make_async_copy(c_hbm, c_v, sm.at[0])
    cp_k = [pltpu.make_async_copy(k_hbm.at[g, pl.ds(SK - W, W), :], k_v.at[g], sk.at[g]) for g in range(HKV)]

    def cp_v(dst, g, sem):
        return pltpu.make_async_copy(v_hbm.at[g, pl.ds(SK - W, W), :],
                                     dst.at[NT + g // 2, pl.ds((g % 2) * W, W), :], sem)

    cp_ve = [cp_v(he_v, g, sv.at[g]) for g in range(1)]
    cp_vo = [cp_v(ho_v, g, sv.at[HKV + g]) for g in range(1)]
    cp_vw = [pltpu.make_async_copy(v_hbm.at[g, pl.ds(SK - W, W), :], wbac_v.at[30, pl.ds(g * W, W), :],
                                   sv.at[2 * HKV + g]) for g in range(HKV)]
    cp_wr = pltpu.make_async_copy(wr_hbm, wr_v, sm.at[3])
    cp_slab_sem = sm.at[4]

    def cp_x(i):
        r0 = pl.multiple_of(i * BM, BM)
        return pltpu.make_async_copy(x_hbm.at[pl.ds(r0, BM), :], x_v.at[pl.ds(r0, BM), :], sx.at[i])

    def cp_out(i):
        r0 = pl.multiple_of(i * BM, BM)
        return pltpu.make_async_copy(out_v.at[pl.ds(r0, BM), :], out_hbm.at[pl.ds(r0, BM), :], so.at[i])

    def cp_tile(w_hbm, w_v, sem, n):
        return pltpu.make_async_copy(w_hbm.at[:, pl.ds(n * 128, 128)], w_v.at[n], sem.at[n])

    cp_wq = functools.partial(cp_tile, wq_hbm, wq_v, swq)
    cp_wo = functools.partial(cp_tile, wo_hbm, wo_v, swo)
    cp_wm = functools.partial(cp_tile, wmod_hbm, wmod_v, swm)
    cp_wg = functools.partial(cp_tile, wg_hbm, wg_v, swg)
    cp_wu = functools.partial(cp_tile, wu_hbm, wu_v, swu)
    cp_wd = functools.partial(cp_tile, wd_hbm, wd_v, swd)

    cp_c.start()
    cp_x(0).start()
    cp_x(1).start()
    cp_c.wait()
    for n in range(2 * NT):
        cp_wm(n).start()
    cc = c_v[...].astype(f32)
    sc16 = jnp.broadcast_to((cc * jax.nn.sigmoid(cc)).astype(bf16), (16, D))

    def mod_tile(n):
        r = jnp.dot(sc16, _b(wmod_u[n]), preferred_element_type=f32)[0:8]
        r = r.astype(bf16).astype(f32)
        if n // NT in (1, 4):
            r = 1.0 + r
        mod_v[n // NT, :, (n % NT) * 128:(n % NT + 1) * 128] = r

    LS = 32

    def normalize(i, dst):
        for o in range(0, BM, LS):
            x = x_v[pl.ds(i * BM + o, LS), :].astype(f32)
            xc = x - jnp.mean(x, axis=-1, keepdims=True)
            dst[o:o + LS, :] = xc * lax.rsqrt(jnp.mean(xc * xc, axis=-1, keepdims=True) + EPS)

    def modulate(src, h_u):
        for o in range(0, BM, LS):
            h = (src[o:o + LS, :] * _rows(mod_v[1], LS) + _rows(mod_v[0], LS)).astype(bf16)
            for kt in range(NT):
                h_u[kt, o // 2:(o + LS) // 2, :] = _u(h[:, kt * 128:(kt + 1) * 128])

    cp_x(0).wait()
    normalize(0, acca_v)
    cp_x(1).wait()
    normalize(1, accb_v)
    for n in range(2 * NT):
        cp_wm(n).wait()
        if n == 11:
            for nn in range(REP):
                cp_wq(nn).start()
            cp_k[0].start()
            cp_ve[0].start()
            cp_vo[0].start()
        mod_tile(n)

    qscale = (DH ** -0.5) * LOG2E

    def ln1(i, h_u, pieces=range(BM // LS)):
        for o in [LS * c for c in pieces]:
            r0 = pl.multiple_of(i * BM + o, LS)
            x = x_v[pl.ds(r0, LS), :].astype(f32)
            h = _ln_mod(x, _rows(mod_v[1], LS), _rows(mod_v[0], LS)).astype(bf16)
            rh = pl.multiple_of(((i // 2) * BM + o) // 2, LS // 2)
            for kt in range(NT):
                h_u[kt, pl.ds(rh, LS // 2), :] = _u(h[:, kt * 128:(kt + 1) * 128])

    def qproj(g, i, h_u, q_dst, js=range(REP)):
        rh = pl.multiple_of((i // 2) * (BM // 2), BM // 2)
        for j in js:
            hh = jnp.concatenate([_b(h_u[kt, pl.ds(rh, BM // 2), :]) for kt in range(NT)], axis=1)
            q = jnp.dot(hh, _b(wq_u[g * REP + j]), preferred_element_type=f32)
            q_dst[j] = _u((q * qscale).astype(bf16))

    def qk(g, q_src, j):
        return lax.dot_general(_b(q_src[j]), _b(k_u[g]), NT_DIMS, preferred_element_type=f32)

    def smpv(g, i, j, s, v_src):
        rh = pl.multiple_of(i * (BM // 2), BM // 2)
        m = jnp.max(s, axis=-1, keepdims=True)
        e = jnp.exp2(s - m)
        l = jnp.sum(e, axis=-1, keepdims=True)
        p = (e * (1.0 / l)).astype(bf16)
        vv = v_src(g)
        o = jnp.dot(p, _b(vv), preferred_element_type=f32)
        o_u[g * REP + j, pl.ds(rh, BM // 2), :] = _u(o.astype(bf16))

    def v_he(g):
        return he_u[NT, 0:W // 2, :]

    def v_ho(g):
        return ho_u[NT, 0:W // 2, :]

    def v_wb(g):
        return wbac_u[30, pl.ds(pl.multiple_of(g * (W // 2), W // 2), W // 2), :]

    def bcombo(gidx):
        gidx = jnp.minimum(gidx, NH * (KH // 16) - 1)
        n = gidx // (KH // 16)
        r = pl.multiple_of((gidx % (KH // 16)) * 8, 8)
        r2 = pl.multiple_of(KH // 2 + r, 8)
        b11 = _b(wo_u[n, pl.ds(r, 8), :]).astype(f32)
        b21 = _b(wo_u[n, pl.ds(r2, 8), :]).astype(f32)
        b12 = _b(wo_u[NH + n, pl.ds(r, 8), :]).astype(f32)
        b22 = _b(wo_u[NH + n, pl.ds(r2, 8), :]).astype(f32)
        for c, val in enumerate((b11 + b22, b12 - b22, b21 - b11, b11 + b12, b21 + b22)):
            wbac_u[c * NH + n, pl.ds(r, 8), :] = _u(val.astype(bf16))

    ALLGROUPS = [(hd, rg) for hd in range(HH) for rg in range(HM // 16)]

    def acombo(i, slot, groups):
        for hd, rg in groups:
            rT = pl.multiple_of(i * HM + rg * 8, 8)
            rB = pl.multiple_of(i * HM + HM // 2 + rg * 8, 8)
            a11 = _b(o_u[hd, pl.ds(rT, 8), :]).astype(f32)
            a12 = _b(o_u[HH + hd, pl.ds(rT, 8), :]).astype(f32)
            a21 = _b(o_u[hd, pl.ds(rB, 8), :]).astype(f32)
            a22 = _b(o_u[HH + hd, pl.ds(rB, 8), :]).astype(f32)
            r = hd * (HM // 2) + rg * 8
            for c, val in enumerate((a11 + a22, a21 + a22, a11 + a12, a21 - a11, a12 - a22)):
                wbac_u[20 + slot * 5 + c, r:r + 8, :] = _u(val.astype(bf16))

    def step(ga, ia, q_src, v_src, gq=None, iq=None, h_u=None, q_dst=None, filler=None, after=False):
        s = qk(ga, q_src, 0)
        for j in range(REP):
            s_next = qk(ga, q_src, j + 1) if j + 1 < REP else None
            if q_dst is not None:
                qproj(gq, iq, h_u, q_dst, [j])
            if filler is not None and not after:
                filler(j)
            smpv(ga, ia, j, s, v_src)
            if filler is not None and after:
                filler(j)
            s = s_next

    modulate(acca_v, he_u)
    modulate(accb_v, ho_u)
    for n in range(0, REP, 2):
        cp_wq(n).wait()
        cp_wq(n + 1).wait()
        qproj(0, 0, he_u, qa_u, [n, n + 1])
    for i in range(2, NB):
        cp_x(i).start()
    for n in range(REP, 2 * REP):
        cp_wq(n).start()
    for g in range(1, HKV):
        cp_k[g].start()
    for g in range(HKV):
        cp_vw[g].start()
    cp_k[0].wait()
    cp_ve[0].wait()
    cp_vo[0].wait()

    def loop1(p, _):
        @pl.when(p == 1)
        def _():
            for n in range(2 * REP, 4 * REP):
                cp_wq(n).start()

        @pl.when(p == 2)
        def _():
            for n in range(NT):
                cp_wo(n).start()
            cp_wr.start()

        @pl.when(p == 3)
        def _():
            for n in range(2 * NT, NMOD):
                cp_wm(n).start()

        @pl.when(p == NB // 2 - 1)
        def _():
            for n in range(REP, 2 * REP):
                cp_wq(n).wait()

        @pl.when(p < NB // 2 - 1)
        def _():
            cp_x(2 * p + 2).wait()
            cp_x(2 * p + 3).wait()

        t = 2 * p
        t2 = t + 2
        step(0, t, qa_u, v_he, 0, t + 1, ho_u, qb_u,
             filler=lambda j: ln1(jnp.minimum(t + 2, NB - 2), he_u, [j]), after=True)
        step(0, t + 1, qb_u, v_ho, t2 // NB, t2 % NB, he_u, qa_u,
             filler=lambda j: ln1(jnp.minimum(t + 3, NB - 1), ho_u, [j]), after=True)
        return 0

    lax.fori_loop(0, NB // 2, loop1, 0)

    for n in range(2 * REP, 4 * REP):
        cp_wq(n).wait()
    for g in range(1, HKV):
        cp_k[g].wait()
    for g in range(HKV):
        cp_vw[g].wait()
    for n in range(NT):
        cp_wo(n).wait()

    NSTEP = HKV * NB

    def loop2(p, _):
        @pl.when(p == 0)
        def _():
            for n in range(NF):
                cp_wg(n).start()

        @pl.when(p == 1)
        def _():
            for n in range(NF):
                cp_wu(n).start()

        @pl.when(p == 2)
        def _():
            for n in range(NT):
                cp_wd(n).start()

        t = NB + 2 * p
        t1, t2 = t + 1, t + 2
        step(t // NB, t % NB, qa_u, v_wb, t1 // NB, t1 % NB, ho_u, qb_u,
             filler=lambda j: [bcombo((p * 2 * REP + j) * 3 + k) for k in range(3)], after=True)
        step(t1 // NB, t1 % NB, qb_u, v_wb, t2 // NB, t2 % NB, he_u, qa_u,
             filler=lambda j: [bcombo((p * 2 * REP + REP + j) * 3 + k) for k in range(3)], after=True)
        return 0

    lax.fori_loop(0, (NSTEP - NB) // 2 - 1, loop2, 0)
    for n in range(2 * NT, NMOD):
        cp_wm(n).wait()
    step(HKV - 1, NB - 2, qa_u, v_wb, HKV - 1, NB - 1, ho_u, qb_u,
         filler=lambda j: acombo(0, 0, ALLGROUPS[j * 16:(j + 1) * 16]), after=True)

    def mod_fill(j):
        for n in range(2 * NT + 4 * j, 2 * NT + 4 * j + 4):
            mod_tile(n)

    step(HKV - 1, NB - 1, qb_u, v_wb, filler=mod_fill)

    cp_wr.wait()
    wr16 = jnp.broadcast_to(wr_v[...], (16, D))

    def lhs(kind, i, slot):
        if kind == "a11":
            r = pl.multiple_of(i * HM, HM // 2)
            return jnp.concatenate([_b(o_u[hd, pl.ds(r, HM // 2), :]) for hd in range(HH)], axis=1)
        if kind == "a22":
            r = pl.multiple_of(i * HM + HM // 2, HM // 2)
            return jnp.concatenate([_b(o_u[HH + hd, pl.ds(r, HM // 2), :]) for hd in range(HH)], axis=1)
        c = {"m1": 0, "m2": 1, "m5": 2, "m6": 3, "m7": 4}[kind]
        return jnp.concatenate(
            [_b(wbac_u[20 + slot * 5 + c, hd * (HM // 2):(hd + 1) * (HM // 2), :]) for hd in range(HH)], axis=1)

    def rhs(kind, n):
        if kind == "b11":
            return _b(wo_u[n, 0:KH // 2, :])
        if kind == "b22":
            return _b(wo_u[NH + n, KH // 2:KH, :])
        return _b(wbac_u[{"m1": 0, "m3": 1, "m4": 2, "m6": 3, "m7": 4}[kind] * NH + n])

    def prod(la, rb, i, slot, n):
        return jnp.dot(lhs(la, i, slot), rhs(rb, n), preferred_element_type=f32)

    def epi(i, acc_r, c0, nc, sub):
        hs = []
        for o in range(0, nc, sub):
            r0 = pl.multiple_of(i * BM + c0 + o, sub)
            x = x_v[pl.ds(r0, sub), :].astype(f32)
            x1 = x + _rows(mod_v[2], sub) * acc_r[c0 + o:c0 + o + sub, :]
            h2 = _ln_mod(x1, _rows(mod_v[4], sub), _rows(mod_v[3], sub))
            h2b = h2.astype(bf16)
            h2_v[pl.ds(r0, sub), :] = h2b
            out_v[pl.ds(r0, sub), :] = (x1 + _rows(mod_v[5], sub) * h2).astype(bf16)
            hs.append(h2b)
        h2b = jnp.concatenate(hs, axis=0) if len(hs) > 1 else hs[0]
        r = lax.dot_general(wr16, h2b, NT_DIMS, preferred_element_type=f32)
        return r[0:8, :].astype(bf16).astype(f32)

    def upd_best(state, i, rs):
        bvv, bii = state
        r = jnp.concatenate(rs, axis=1)
        rows = i * BM + lax.broadcasted_iota(jnp.int32, (8, BM), 1)
        upd = r > bvv
        return jnp.where(upd, r, bvv), jnp.where(upd, rows, bii)

    def half(i, slot, acc_w, i_prev, acc_r, state, inext=None, snext=None, do_epi=True):
        rs = []
        per = len(ALLGROUPS) // (NH * 7)
        extra = len(ALLGROUPS) - per * NH * 7
        pos = [0, 0]

        def fill():
            cnt = per + (1 if pos[1] < extra else 0)
            if inext is not None:
                acombo(inext, snext, ALLGROUPS[pos[0]:pos[0] + cnt])
            pos[0] += cnt
            pos[1] += 1

        for n in range(NH):
            c22 = prod("m6", "m6", i, slot, n)
            fill()
            m3 = prod("a11", "m3", i, slot, n)
            fill()
            c22 = c22 + m3
            m5 = prod("m5", "b22", i, slot, n)
            fill()
            acc_w[0:HM, (NH + n) * 128:(NH + n + 1) * 128] = m3 + m5
            c11 = prod("m7", "m7", i, slot, n) - m5
            fill()
            m1 = prod("m1", "m1", i, slot, n)
            fill()
            c11 = c11 + m1
            c22 = c22 + m1
            m4 = prod("a22", "m4", i, slot, n)
            fill()
            acc_w[0:HM, n * 128:(n + 1) * 128] = c11 + m4
            m2 = prod("m2", "b11", i, slot, n)
            fill()
            acc_w[HM:BM, n * 128:(n + 1) * 128] = m4 + m2
            acc_w[HM:BM, (NH + n) * 128:(NH + n + 1) * 128] = c22 - m2
            if do_epi and n in (1, 3):
                rs.append(epi(i_prev, acc_r, (n // 2) * HM, HM, SUB))
        if do_epi:
            state = upd_best(state, i_prev, rs)
            cp_out(i_prev).start()
        return state

    state = (jnp.full((8, BM), -jnp.inf, f32), jnp.zeros((8, BM), jnp.int32))
    half(0, 0, acca_v, None, None, state, 1, 1, do_epi=False)

    def loopb(p, state):
        i = 2 * p
        state = half(i + 1, 1, accb_v, i, acca_v, state, i + 2, 0)
        state = half(i + 2, 0, acca_v, i + 1, accb_v, state, i + 3, 1)
        return state

    state = lax.fori_loop(0, NB // 2 - 1, loopb, state)
    for n in range(NF):
        cp_wg(n).wait()
        cp_wu(n).wait()
    for n in range(NT):
        cp_wd(n).wait()
    state = half(NB - 1, 1, accb_v, NB - 2, acca_v, state)
    rs = [epi(NB - 1, accb_v, c * 128, 128, 64) for c in range(BM // 128)]
    best_v, best_i = upd_best(state, NB - 1, rs)
    cp_out(NB - 1).start()

    rmax = jnp.max(best_v, axis=1, keepdims=True)
    idx = jnp.min(jnp.where(best_v == rmax, best_i, S), axis=1, keepdims=True)
    idx_s = idx[0, 0]
    base = pl.multiple_of((idx_s // 16) * 16, 16)
    hs = h2_v[pl.ds(base, 16), :]
    acts = []
    for n in range(NF):
        gg = jnp.dot(hs, _b(wg_u[n]), preferred_element_type=f32).astype(bf16).astype(f32)
        uu = jnp.dot(hs, _b(wu_u[n]), preferred_element_type=f32).astype(bf16).astype(f32)
        acts.append(((gg * jax.nn.sigmoid(gg)).astype(bf16).astype(f32) * uu).astype(bf16))
    act = jnp.concatenate(acts, axis=1)
    old = out_v[pl.ds(base, 16), :].astype(f32)
    rowi = base + lax.broadcasted_iota(jnp.int32, (16, 1), 0)
    sig = jax.nn.sigmoid(rmax[0:1, :])
    sel = rowi == idx[0:1, :]
    for n in range(NT):
        y = jnp.dot(act, _b(wd_u[n]), preferred_element_type=f32).astype(bf16).astype(f32)
        new = old[:, n * 128:(n + 1) * 128] + _rows(mod_v[5, :, n * 128:(n + 1) * 128], 16) * (y * sig)
        slab_v[:, n * 128:(n + 1) * 128] = jnp.where(sel, new, old[:, n * 128:(n + 1) * 128]).astype(bf16)
    for i in range(NB):
        cp_out(i).wait()
    cp_slab = pltpu.make_async_copy(slab_v, out_hbm.at[pl.ds(base, 16), :], cp_slab_sem)
    cp_slab.start()
    cp_slab.wait()


@jax.jit
def pallas_adaLN_cond__sliding_block_cached__moe_arch_mod__prompt_kernel(
        A_x, A_k_cache, A_v_cache, A_wq, A_wo, B_x, B_w_r, B_w_gate, B_w_up, B_w_down, c, w_mod):
    x = A_x.reshape(S, D)
    k = A_k_cache.reshape(HKV, SK, DH)
    v = A_v_cache.reshape(HKV, SK, DH)
    wr = B_w_r.reshape(1, D)
    anyspec = pl.BlockSpec(memory_space=pl.ANY)
    out = pl.pallas_call(
        kernel,
        out_shape=jax.ShapeDtypeStruct((S, D), bf16),
        in_specs=[anyspec] * 11,
        out_specs=anyspec,
        scratch_shapes=[
            pltpu.VMEM((3, S, D), bf16),
            pltpu.VMEM((HKV, W, DH), bf16),
            pltpu.VMEM((HQ, D, 128), bf16),
            pltpu.VMEM((NT, HQ * DH, 128), bf16),
            pltpu.VMEM((1, D), bf16),
            pltpu.VMEM((NF, D, 128), bf16),
            pltpu.VMEM((NF, D, 128), bf16),
            pltpu.VMEM((NT, F, 128), bf16),
            pltpu.VMEM((1, D), bf16),
            pltpu.VMEM((NMOD, D, 128), bf16),
            pltpu.VMEM((NT + 1, S // 2, 128), bf16),
            pltpu.VMEM((NT + 1, S // 2, 128), bf16),
            pltpu.VMEM((HQ, S, 128), bf16),
            pltpu.VMEM((REP, BM, 128), bf16),
            pltpu.VMEM((REP, BM, 128), bf16),
            pltpu.VMEM((6, 8, D), f32),
            pltpu.VMEM((31, KH, 128), bf16),
            pltpu.VMEM((BM, D), f32),
            pltpu.VMEM((BM, D), f32),
            pltpu.VMEM((16, D), bf16),
            pltpu.SemaphoreType.DMA((NB,)),
            pltpu.SemaphoreType.DMA((HQ,)),
            pltpu.SemaphoreType.DMA((NT,)),
            pltpu.SemaphoreType.DMA((NMOD,)),
            pltpu.SemaphoreType.DMA((NF,)),
            pltpu.SemaphoreType.DMA((NF,)),
            pltpu.SemaphoreType.DMA((NT,)),
            pltpu.SemaphoreType.DMA((NB,)),
            pltpu.SemaphoreType.DMA((3 * HKV,)),
            pltpu.SemaphoreType.DMA((HKV,)),
            pltpu.SemaphoreType.DMA((5,)),
        ],
        compiler_params=pltpu.CompilerParams(vmem_limit_bytes=120 * 1024 * 1024),
    )(x, k, v, A_wq, A_wo, wr, B_w_gate, B_w_up, B_w_down, c, w_mod)
    return out.reshape(1, S, D)
```

```python
import functools

import jax
import jax.numpy as jnp
from jax import lax
import jax.experimental.pallas as pl
import jax.experimental.pallas.tpu as pltpu

S, D = 2048, 1024
HQ, HKV, DH = 32, 4, 128
SK = 2048
W = 512
REP = HQ // HKV
F = 3584
EPS = 1e-5
LOG2E = 1.4426950408889634
BM = 256
NB = S // BM
HM = BM // 2
NT = D // 128
NF = F // 128
NMOD = 6 * NT
SUB = 16
KH = HQ * DH // 2
NH = NT // 2
HH = HQ // 2
QH = D // 2
QT = QH // 128
NP = REP // 2
WB_WO, WB_AC, WB_V = 0, 20, 30
WB_SLOTS = 31
WQC_V = HKV * NP * 5
HC = {"m1": 0, "m2": 1, "m3": 2, "m4": 3, "m5": 4, "m6": 5, "m7": 6}
WC = {"m1": 0, "m3": 1, "m4": 2, "m6": 3, "m7": 4}
AC = {"m1": 0, "m2": 1, "m5": 2, "m6": 3, "m7": 4}

f32 = jnp.float32
bf16 = jnp.bfloat16
u32 = jnp.uint32
NT_DIMS = (((1,), (1,)), ((), ()))


def _rows(m8, n):
    return jnp.concatenate([m8] * (n // 8), axis=0) if n > 8 else m8


def _normalize(x):
    xc = x - jnp.mean(x, axis=-1, keepdims=True)
    return xc * lax.rsqrt(jnp.mean(xc * xc, axis=-1, keepdims=True) + EPS)


def _b(u):
    return pltpu.bitcast(u, bf16)


def _u(b):
    return pltpu.bitcast(b, u32)


def _kernel(x_hbm, k_hbm, v_hbm, wq_hbm, wo_hbm, wr_hbm, wg_hbm, wu_hbm, wd_hbm, c_hbm, wmod_hbm,
            out_hbm,
            xo_v, k_v, wq_v, wo_v, wr_v, wg_v, wu_v, wd_v, c_v, wmod_v,
            hce_v, hco_v, o_v, qa_v, qb_v, mod_v, wb_v, wqc_v, acca_v, accb_v, slab_v,
            sx, swq, swo, swm, swg, swu, swd, so, sv, sk, sm):
    x_v = xo_v.at[0]
    h2_v = xo_v.at[1]
    out_v = xo_v.at[2]
    k_u = k_v.bitcast(u32)
    wq_u = wq_v.bitcast(u32)
    wo_u = wo_v.bitcast(u32)
    wg_u = wg_v.bitcast(u32)
    wu_u = wu_v.bitcast(u32)
    wd_u = wd_v.bitcast(u32)
    wmod_u = wmod_v.bitcast(u32)
    hce_u = hce_v.bitcast(u32)
    hco_u = hco_v.bitcast(u32)
    o_u = o_v.bitcast(u32)
    qa_u = qa_v.bitcast(u32)
    qb_u = qb_v.bitcast(u32)
    wb_u = wb_v.bitcast(u32)
    wqc_u = wqc_v.bitcast(u32)

    cp_c = pltpu.make_async_copy(c_hbm, c_v, sm.at[0])
    cp_wr = pltpu.make_async_copy(wr_hbm, wr_v, sm.at[1])
    win = pl.ds(SK - W, W)
    cp_k = [pltpu.make_async_copy(k_hbm.at[g, win, :], k_v.at[g], sk.at[g])
            for g in range(HKV)]
    cp_v = [pltpu.make_async_copy(v_hbm.at[g, win, :], wb_v.at[WB_V, pl.ds(g * W, W), :], sv.at[g])
            for g in range(HKV)]
    cp_vq = [pltpu.make_async_copy(v_hbm.at[g, win, :], wqc_v.at[WQC_V + g], sv.at[HKV + 2 + g])
             for g in range(HKV)]
    cp_ve = pltpu.make_async_copy(v_hbm.at[0, win, :], hce_v.at[7 * QT], sv.at[HKV])
    cp_vo = pltpu.make_async_copy(v_hbm.at[0, win, :], hco_v.at[7 * QT], sv.at[HKV + 1])

    def cp_x(i):
        r = pl.ds(pl.multiple_of(i * BM, BM), BM)
        return pltpu.make_async_copy(x_hbm.at[r, :], x_v.at[r, :], sx.at[i])

    def cp_out(i):
        r = pl.ds(pl.multiple_of(i * BM, BM), BM)
        return pltpu.make_async_copy(out_v.at[r, :], out_hbm.at[r, :], so.at[i])

    def cp_tile(w_hbm, w_v, sem, n):
        return pltpu.make_async_copy(w_hbm.at[:, pl.ds(n * 128, 128)], w_v.at[n], sem.at[n])

    cp_wq = functools.partial(cp_tile, wq_hbm, wq_v, swq)
    cp_wo = functools.partial(cp_tile, wo_hbm, wo_v, swo)
    cp_wm = functools.partial(cp_tile, wmod_hbm, wmod_v, swm)
    cp_wg = functools.partial(cp_tile, wg_hbm, wg_v, swg)
    cp_wu = functools.partial(cp_tile, wu_hbm, wu_v, swu)
    cp_wd = functools.partial(cp_tile, wd_hbm, wd_v, swd)

    cp_c.start()
    cp_x(0).start()
    cp_x(1).start()
    cp_c.wait()
    for n in range(2 * NT):
        cp_wm(n).start()
    cc = c_v[...].astype(f32)
    sc16 = jnp.broadcast_to((cc * jax.nn.sigmoid(cc)).astype(bf16), (16, D))

    def mod_tile(n):
        r = jnp.dot(sc16, _b(wmod_u[n]), preferred_element_type=f32)[0:8]
        r = r.astype(bf16).astype(f32)
        if n // NT in (1, 4):
            r = 1.0 + r
        mod_v[n // NT, :, (n % NT) * 128:(n % NT + 1) * 128] = r

    def store_hc(h, hc_v, r):
        ht, hb = h[:16], h[16:]
        a11, a12, a21, a22 = ht[:, :QH], ht[:, QH:], hb[:, :QH], hb[:, QH:]
        combos = (a11 + a22, a21 + a22, a11, a22, a11 + a12, a21 - a11, a12 - a22)
        for ci, val in enumerate(combos):
            vb = val.astype(bf16)
            for kt in range(QT):
                hc_v[ci * QT + kt, r, :] = vb[:, kt * 128:(kt + 1) * 128]

    def piece_rows(i, c):
        return (pl.ds(pl.multiple_of(i * BM + 16 * c, 16), 16),
                pl.ds(pl.multiple_of(i * BM + HM + 16 * c, 16), 16))

    def ln1_piece(i, hc_v, c):
        rt, rb = piece_rows(i, c)
        x = jnp.concatenate([x_v[rt, :], x_v[rb, :]], axis=0).astype(f32)
        h = _normalize(x) * _rows(mod_v[1], 32) + _rows(mod_v[0], 32)
        store_hc(h, hc_v, pl.ds(pl.multiple_of((i // 2) * HM + 16 * c, 16), 16))

    def normalize_block(i, dst):
        for c in range(HM // 16):
            rt, rb = 16 * c, HM + 16 * c
            x = jnp.concatenate([x_v[i * BM + rt:i * BM + rt + 16, :], x_v[i * BM + rb:i * BM + rb + 16, :]], axis=0)
            dst[32 * c:32 * c + 32, :] = _normalize(x.astype(f32))

    def modulate_block(src, hc_v):
        for c in range(HM // 16):
            h = src[32 * c:32 * c + 32, :] * _rows(mod_v[1], 32) + _rows(mod_v[0], 32)
            store_hc(h, hc_v, pl.ds(16 * c, 16))

    cp_x(0).wait()
    normalize_block(0, acca_v)
    cp_x(1).wait()
    normalize_block(1, accb_v)
    wq_first = [j + NP * hi for j in range(NP) for hi in range(2)]
    for n in range(2 * NT):
        cp_wm(n).wait()
        if n == 11:
            for nn in wq_first:
                cp_wq(nn).start()
            cp_k[0].start()
            cp_ve.start()
            cp_vo.start()
        mod_tile(n)

    def wq_combo(grp):
        pair = grp // 8
        r0 = pl.multiple_of((grp % 8) * 32, 32)
        lo = (pair // NP) * REP + pair % NP
        t0 = pair * 5
        for k in range(4):
            r = pl.ds(pl.multiple_of(r0 + 8 * k, 8), 8)
            r2 = pl.ds(pl.multiple_of(r0 + (QH // 2 + 8 * k), 8), 8)
            b11 = _b(wq_u[lo, r, :]).astype(f32)
            b21 = _b(wq_u[lo, r2, :]).astype(f32)
            b12 = _b(wq_u[lo + NP, r, :]).astype(f32)
            b22 = _b(wq_u[lo + NP, r2, :]).astype(f32)
            for ci, val in enumerate((b11 + b22, b12 - b22, b21 - b11, b11 + b12, b21 + b22)):
                wqc_v[t0 + ci, pl.ds(pl.multiple_of(2 * r0 + 16 * k, 16), 16), :] = val.astype(bf16)

    def wo_combo(grp):
        n = grp // (KH // 64)
        r0 = pl.multiple_of((grp % (KH // 64)) * 32, 32)
        for k in range(4):
            r = pl.ds(pl.multiple_of(r0 + 8 * k, 8), 8)
            r2 = pl.ds(pl.multiple_of(r0 + (KH // 2 + 8 * k), 8), 8)
            b11 = _b(wo_u[n, r, :]).astype(f32)
            b21 = _b(wo_u[n, r2, :]).astype(f32)
            b12 = _b(wo_u[NH + n, r, :]).astype(f32)
            b22 = _b(wo_u[NH + n, r2, :]).astype(f32)
            for ci, val in enumerate((b11 + b22, b12 - b22, b21 - b11, b11 + b12, b21 + b22)):
                wb_v[WB_WO + ci * NH + n, pl.ds(pl.multiple_of(2 * r0 + 16 * k, 16), 16), :] = val.astype(bf16)

    GQ = NP * 8
    NWO = NH * (KH // 64)

    qscale = (DH ** -0.5) * LOG2E

    def qprod(name, g, i, hc_u, jp):
        r = pl.ds(pl.multiple_of((i // 2) * (HM // 2), HM // 2), HM // 2)
        a = jnp.concatenate([_b(hc_u[HC[name] * QT + kt, r, :]) for kt in range(QT)], axis=1)
        if name == "m2":
            b = wq_u[g * REP + jp, 0:QH // 2, :]
        elif name == "m5":
            b = wq_u[g * REP + jp + NP, QH // 2:QH, :]
        else:
            b = wqc_u[(g * NP + jp) * 5 + WC[name]]
        return jnp.dot(a, _b(b), preferred_element_type=f32)

    def qstore(q_dst, j, half, val):
        q_dst[j, half * HM:(half + 1) * HM, :] = (val * qscale).astype(bf16)

    def qproj_part(g, i, hc_u, q_dst, jp, part, carry):
        prod = lambda name: qprod(name, g, i, hc_u, jp)
        if part == 0:
            c22 = prod("m6")
            m3 = prod("m3")
            c22 = c22 + m3
            m5 = prod("m5")
            qstore(q_dst, jp + NP, 0, m3 + m5)
            return prod("m7") - m5, c22
        c11, c22 = carry
        m1 = prod("m1")
        c11 = c11 + m1
        c22 = c22 + m1
        m4 = prod("m4")
        qstore(q_dst, jp, 0, c11 + m4)
        m2 = prod("m2")
        qstore(q_dst, jp, 1, m4 + m2)
        qstore(q_dst, jp + NP, 1, c22 - m2)
        return None

    def kv_rows(g):
        return pl.ds(pl.multiple_of(g * (W // 2), W // 2), W // 2)

    def qk(g, q_src, j):
        return lax.dot_general(_b(q_src[j]), _b(k_u[g]), NT_DIMS, preferred_element_type=f32)

    def softmax_pv(g, i, j, s, v_src):
        m = jnp.max(s, axis=-1, keepdims=True)
        e = jnp.exp2(s - m)
        l = jnp.sum(e, axis=-1, keepdims=True)
        p = (e * (1.0 / l)).astype(bf16)
        o = jnp.dot(p, _b(v_src(g)), preferred_element_type=f32)
        o_v[g * REP + j, pl.ds(pl.multiple_of(i * BM, BM), BM), :] = o.astype(bf16)

    v_wb = lambda g: wb_u[WB_V, kv_rows(g), :]
    v_wq = lambda g: wqc_u[WQC_V + g]
    v_he = lambda g: hce_u[7 * QT]
    v_ho = lambda g: hco_u[7 * QT]

    def step(ga, ia, q_src, v_src, gq=None, iq=None, hc_u=None, q_dst=None, before=None, after=None):
        s = qk(ga, q_src, 0)
        carry = None
        for j in range(REP):
            s_next = qk(ga, q_src, j + 1) if j + 1 < REP else None
            if q_dst is not None:
                carry = qproj_part(gq, iq, hc_u, q_dst, j // 2, j % 2, carry)
            if before is not None:
                before(j)
            softmax_pv(ga, ia, j, s, v_src)
            if after is not None:
                after(j)
            s = s_next

    modulate_block(acca_v, hce_v)
    modulate_block(accb_v, hco_v)
    for jp in range(NP):
        cp_wq(jp).wait()
        cp_wq(jp + NP).wait()
        if jp == 1:
            cp_x(2).start()
            cp_x(3).start()
        for grp in range(jp * 8, (jp + 1) * 8):
            wq_combo(grp)
        carry = qproj_part(0, 0, hce_u, qa_v, jp, 0, None)
        qproj_part(0, 0, hce_u, qa_v, jp, 1, carry)
    for i in range(4, NB):
        cp_x(i).start()
    for n in range(REP, 2 * REP):
        cp_wq(n).start()
    for g in range(1, HKV):
        cp_k[g].start()
    for g in range(HKV):
        cp_v[g].start()
        cp_vq[g].start()
    cp_k[0].wait()
    cp_ve.wait()
    cp_vo.wait()

    def loop1(p, _):
        @pl.when(p == 1)
        def _():
            for n in range(REP, 2 * REP):
                cp_wq(n).wait()
            for n in range(2 * REP, 4 * REP):
                cp_wq(n).start()

        @pl.when(p == 2)
        def _():
            for n in range(NT):
                cp_wo(n).start()
            cp_wr.start()

        @pl.when(p == 3)
        def _():
            for n in range(2 * NT, NMOD):
                cp_wm(n).start()

        @pl.when(p < NB // 2 - 1)
        def _():
            cp_x(2 * p + 2).wait()
            cp_x(2 * p + 3).wait()

        @pl.when(p == 2)
        def _():
            for grp in range(GQ, 2 * GQ):
                wq_combo(grp)

        t = 2 * p
        t2 = t + 2
        ia, ib = jnp.minimum(t + 2, NB - 2), jnp.minimum(t + 3, NB - 1)
        step(0, t, qa_u, v_he, 0, t + 1, hco_u, qb_v, after=lambda j: ln1_piece(ia, hce_v, j))
        step(0, t + 1, qb_u, v_ho, t2 // NB, t2 % NB, hce_u, qa_v, after=lambda j: ln1_piece(ib, hco_v, j))
        return 0

    lax.fori_loop(0, NB // 2, loop1, 0)

    for n in range(2 * REP, 4 * REP):
        cp_wq(n).wait()
    for g in range(1, HKV):
        cp_k[g].wait()
    for g in range(HKV):
        cp_v[g].wait()
        cp_vq[g].wait()
    for n in range(NT):
        cp_wo(n).wait()

    NSTEP = HKV * NB

    def loop2(p, _):
        @pl.when(p == 0)
        def _():
            for n in range(NF):
                cp_wg(n).start()

        @pl.when(p == 1)
        def _():
            for n in range(NF):
                cp_wu(n).start()

        @pl.when(p == 2)
        def _():
            for n in range(NT):
                cp_wd(n).start()

        t = NB + 2 * p
        t1, t2 = t + 1, t + 2
        grp = 2 * GQ + p * 2 * REP
        step(t // NB, t % NB, qa_u, v_wq, t1 // NB, t1 % NB, hco_u, qb_v, after=lambda j: wq_combo(grp + j))
        step(t1 // NB, t1 % NB, qb_u, v_wq, t2 // NB, t2 % NB, hce_u, qa_v,
             after=lambda j: wq_combo(grp + REP + j))
        return 0

    NA = 2 * GQ // (2 * REP)

    lax.fori_loop(0, NA, loop2, 0)

    def loop3(p, _):
        t = NB + 2 * (NA + p)
        t1, t2 = t + 1, t + 2
        grp = p * 2 * REP
        step(t // NB, t % NB, qa_u, v_wb, t1 // NB, t1 % NB, hco_u, qb_v, after=lambda j: wo_combo(grp + j))
        step(t1 // NB, t1 % NB, qb_u, v_wb, t2 // NB, t2 % NB, hce_u, qa_v,
             after=lambda j: wo_combo(grp + REP + j))
        return 0

    NC = (NSTEP - NB) // 2 - 1 - NA
    lax.fori_loop(0, NC, loop3, 0)
    WO_DONE = NC * 2 * REP

    ac_jobs = [(hd, rg) for hd in range(HH) for rg in range(HM // 16)]

    def a_combo(i, slot, jobs):
        for hd, rg in jobs:
            rt = pl.ds(pl.multiple_of(i * HM + rg * 8, 8), 8)
            rb = pl.ds(pl.multiple_of(i * HM + HM // 2 + rg * 8, 8), 8)
            a11 = _b(o_u[hd, rt, :]).astype(f32)
            a12 = _b(o_u[HH + hd, rt, :]).astype(f32)
            a21 = _b(o_u[hd, rb, :]).astype(f32)
            a22 = _b(o_u[HH + hd, rb, :]).astype(f32)
            r = hd * HM + rg * 16
            for ci, val in enumerate((a11 + a22, a21 + a22, a11 + a12, a21 - a11, a12 - a22)):
                wb_v[WB_AC + slot * 5 + ci, r:r + 16, :] = val.astype(bf16)

    cp_wr.wait()
    wr16 = jnp.broadcast_to(wr_v[...], (16, D))

    def olhs(kind, i, slot):
        if kind == "m3":
            r = pl.ds(pl.multiple_of(i * HM, HM // 2), HM // 2)
            return jnp.concatenate([_b(o_u[hd, r, :]) for hd in range(HH)], axis=1)
        if kind == "m4":
            r = pl.ds(pl.multiple_of(i * HM + HM // 2, HM // 2), HM // 2)
            return jnp.concatenate([_b(o_u[HH + hd, r, :]) for hd in range(HH)], axis=1)
        return jnp.concatenate(
            [_b(wb_u[WB_AC + slot * 5 + AC[kind], hd * (HM // 2):(hd + 1) * (HM // 2), :]) for hd in range(HH)],
            axis=1)

    def orhs(kind, n):
        if kind == "m2":
            return _b(wo_u[n, 0:KH // 2, :])
        if kind == "m5":
            return _b(wo_u[NH + n, KH // 2:KH, :])
        return _b(wb_u[WB_WO + WC[kind] * NH + n])

    def oprod(kind, i, slot, n):
        return jnp.dot(olhs(kind, i, slot), orhs(kind, n), preferred_element_type=f32)

    def epilogue(i, acc_r, c0, nc, sub):
        hs = []
        for o in range(0, nc, sub):
            r = pl.ds(pl.multiple_of(i * BM + c0 + o, sub), sub)
            x1 = x_v[r, :].astype(f32) + _rows(mod_v[2], sub) * acc_r[c0 + o:c0 + o + sub, :]
            h2 = _normalize(x1) * _rows(mod_v[4], sub) + _rows(mod_v[3], sub)
            h2b = h2.astype(bf16)
            h2_v[r, :] = h2b
            out_v[r, :] = (x1 + _rows(mod_v[5], sub) * h2).astype(bf16)
            hs.append(h2b)
        h2b = jnp.concatenate(hs, axis=0) if len(hs) > 1 else hs[0]
        score = lax.dot_general(wr16, h2b, NT_DIMS, preferred_element_type=f32)
        return score[0:8, :].astype(bf16).astype(f32)

    def update_best(state, i, scores):
        best_v, best_i = state
        r = jnp.concatenate(scores, axis=1)
        rows = i * BM + lax.broadcasted_iota(jnp.int32, (8, BM), 1)
        better = r > best_v
        return jnp.where(better, r, best_v), jnp.where(better, rows, best_i)

    def block_steps(i, slot, acc_w, i_prev, acc_r, result, inext=None, snext=None, do_epi=True):
        scores = []
        nprod = NH * 7
        per = len(ac_jobs) // nprod
        extra = len(ac_jobs) - per * nprod
        pos = [0, 0]

        def fill():
            cnt = per + (1 if pos[1] < extra else 0)
            if inext is not None:
                a_combo(inext, snext, ac_jobs[pos[0]:pos[0] + cnt])
            pos[0] += cnt
            pos[1] += 1

        def prod(kind, n):
            val = oprod(kind, i, slot, n)
            fill()
            return val

        def fill_only():
            fill()

        for n in range(NH):
            cl = slice(n * 128, (n + 1) * 128)
            cr = slice((NH + n) * 128, (NH + n + 1) * 128)
            c22 = prod("m6", n)
            yield
            m3 = prod("m3", n)
            yield
            c22 = c22 + m3
            m5 = prod("m5", n)
            yield
            acc_w[0:HM, cr] = m3 + m5
            c11 = prod("m7", n) - m5
            yield
            m1 = prod("m1", n)
            yield
            c11 = c11 + m1
            c22 = c22 + m1
            m4 = prod("m4", n)
            yield
            acc_w[0:HM, cl] = c11 + m4
            m2 = prod("m2", n)
            acc_w[HM:BM, cl] = m4 + m2
            acc_w[HM:BM, cr] = c22 - m2
            if do_epi and n in (1, 3):
                scores.append(epilogue(i_prev, acc_r, (n // 2) * HM, HM, SUB))
            if n < NH - 1:
                yield
        if do_epi:
            result[0] = update_best(result[0], i_prev, scores)
            cp_out(i_prev).start()

    def block(i, slot, acc_w, i_prev, acc_r, state, inext=None, snext=None):
        result = [state]
        for _ in block_steps(i, slot, acc_w, i_prev, acc_r, result, inext, snext):
            pass
        return result[0]

    for n in range(2 * NT, NMOD):
        cp_wm(n).wait()
    step(HKV - 1, NB - 2, qa_u, v_wb, HKV - 1, NB - 1, hco_u, qb_v,
         after=lambda j: (wo_combo(WO_DONE + 2 * j), wo_combo(WO_DONE + 2 * j + 1),
                          a_combo(0, 0, ac_jobs[j * 16:(j + 1) * 16])))

    first = block_steps(0, 0, acca_v, None, None, None, 1, 1, do_epi=False)

    def first_fill(j):
        for n in range(2 * NT + 4 * j, 2 * NT + 4 * j + 4):
            mod_tile(n)
        for _ in range(4 if j % 2 else 3):
            next(first, None)

    step(HKV - 1, NB - 1, qb_u, v_wb, before=first_fill)
    for _ in first:
        pass

    state = (jnp.full((8, BM), -jnp.inf, f32), jnp.zeros((8, BM), jnp.int32))

    def loopb(p, state):
        i = 2 * p
        state = block(i + 1, 1, accb_v, i, acca_v, state, i + 2, 0)
        state = block(i + 2, 0, acca_v, i + 1, accb_v, state, i + 3, 1)
        return state

    state = lax.fori_loop(0, NB // 2 - 1, loopb, state)
    for n in range(NF):
        cp_wg(n).wait()
        cp_wu(n).wait()
    for n in range(NT):
        cp_wd(n).wait()
    state = block(NB - 1, 1, accb_v, NB - 2, acca_v, state)
    scores = [epilogue(NB - 1, accb_v, c * 128, 128, 64) for c in range(BM // 128)]
    best_v, best_i = update_best(state, NB - 1, scores)
    cp_out(NB - 1).start()

    rmax = jnp.max(best_v, axis=1, keepdims=True)
    idx = jnp.min(jnp.where(best_v == rmax, best_i, S), axis=1, keepdims=True)
    base = pl.multiple_of((idx[0, 0] // 16) * 16, 16)
    hs = h2_v[pl.ds(base, 16), :]
    acts = []
    for n in range(NF):
        gate = jnp.dot(hs, _b(wg_u[n]), preferred_element_type=f32).astype(bf16).astype(f32)
        up = jnp.dot(hs, _b(wu_u[n]), preferred_element_type=f32).astype(bf16).astype(f32)
        acts.append(((gate * jax.nn.sigmoid(gate)).astype(bf16).astype(f32) * up).astype(bf16))
    act = jnp.concatenate(acts, axis=1)
    old = out_v[pl.ds(base, 16), :].astype(f32)
    sel = base + lax.broadcasted_iota(jnp.int32, (16, 1), 0) == idx[0:1, :]
    weight = jax.nn.sigmoid(rmax[0:1, :])
    for n in range(NT):
        cols = slice(n * 128, (n + 1) * 128)
        y = jnp.dot(act, _b(wd_u[n]), preferred_element_type=f32).astype(bf16).astype(f32)
        new = old[:, cols] + _rows(mod_v[5, :, cols], 16) * (y * weight)
        slab_v[:, cols] = jnp.where(sel, new, old[:, cols]).astype(bf16)
    for i in range(NB):
        cp_out(i).wait()
    cp_slab = pltpu.make_async_copy(slab_v, out_hbm.at[pl.ds(base, 16), :], sm.at[2])
    cp_slab.start()
    cp_slab.wait()


@jax.jit
def pallas_adaLN_cond__sliding_block_cached__moe_arch_mod__prompt_kernel(
        A_x, A_k_cache, A_v_cache, A_wq, A_wo, B_x, B_w_r, B_w_gate, B_w_up, B_w_down, c, w_mod):
    x = A_x.reshape(S, D)
    k = A_k_cache.reshape(HKV, SK, DH)
    v = A_v_cache.reshape(HKV, SK, DH)
    wr = B_w_r.reshape(1, D)
    anyspec = pl.BlockSpec(memory_space=pl.ANY)
    dma = pltpu.SemaphoreType.DMA
    out = pl.pallas_call(
        _kernel,
        out_shape=jax.ShapeDtypeStruct((S, D), bf16),
        in_specs=[anyspec] * 11,
        out_specs=anyspec,
        scratch_shapes=[
            pltpu.VMEM((3, S, D), bf16),
            pltpu.VMEM((HKV, W, DH), bf16),
            pltpu.VMEM((HQ, D, 128), bf16),
            pltpu.VMEM((NT, HQ * DH, 128), bf16),
            pltpu.VMEM((1, D), bf16),
            pltpu.VMEM((NF, D, 128), bf16),
            pltpu.VMEM((NF, D, 128), bf16),
            pltpu.VMEM((NT, F, 128), bf16),
            pltpu.VMEM((1, D), bf16),
            pltpu.VMEM((NMOD, D, 128), bf16),
            pltpu.VMEM((7 * QT + 1, S // 4, 128), bf16),
            pltpu.VMEM((7 * QT + 1, S // 4, 128), bf16),
            pltpu.VMEM((HQ, S, 128), bf16),
            pltpu.VMEM((REP, BM, 128), bf16),
            pltpu.VMEM((REP, BM, 128), bf16),
            pltpu.VMEM((6, 8, D), f32),
            pltpu.VMEM((WB_SLOTS, KH, 128), bf16),
            pltpu.VMEM((WQC_V + HKV, QH, 128), bf16),
            pltpu.VMEM((BM, D), f32),
            pltpu.VMEM((BM, D), f32),
            pltpu.VMEM((16, D), bf16),
            dma((NB,)), dma((HQ,)), dma((NT,)), dma((NMOD,)), dma((NF,)), dma((NF,)), dma((NT,)),
            dma((NB,)), dma((2 * HKV + 2,)), dma((HKV,)), dma((3,)),
        ],
        compiler_params=pltpu.CompilerParams(vmem_limit_bytes=124 * 1024 * 1024),
    )(x, k, v, A_wq, A_wo, wr, B_w_gate, B_w_up, B_w_down, c, w_mod)
    return out.reshape(1, S, D)
```

```python
import functools

import jax
import jax.numpy as jnp
from jax import lax
import jax.experimental.pallas as pl
import jax.experimental.pallas.tpu as pltpu

S, D = 2048, 1024
HQ, HKV, DH = 32, 4, 128
SK = 2048
W = 512
REP = HQ // HKV
F = 3584
EPS = 1e-5
LOG2E = 1.4426950408889634
BM = 256
NB = S // BM
HM = BM // 2
NT = D // 128
NF = F // 128
NMOD = 6 * NT
SUB = 16
KH = HQ * DH // 2
NH = NT // 2
HH = HQ // 2
QH = D // 2
QT = QH // 128
NP = REP // 2
WB_WO, WB_AC, WB_V = 0, 20, 30
WB_SLOTS = 31
WQC_V = HKV * NP * 5
HC = {"m1": 0, "m2": 1, "m3": 2, "m4": 3, "m5": 4, "m6": 5, "m7": 6}
WC = {"m1": 0, "m3": 1, "m4": 2, "m6": 3, "m7": 4}
AC = {"m1": 0, "m2": 1, "m5": 2, "m6": 3, "m7": 4}

f32 = jnp.float32
bf16 = jnp.bfloat16
u32 = jnp.uint32
NT_DIMS = (((1,), (1,)), ((), ()))


def _rows(m8, n):
    return jnp.concatenate([m8] * (n // 8), axis=0) if n > 8 else m8


def _normalize(x):
    xc = x - jnp.mean(x, axis=-1, keepdims=True)
    return xc * lax.rsqrt(jnp.mean(xc * xc, axis=-1, keepdims=True) + EPS)


def _b(u):
    return pltpu.bitcast(u, bf16)


def _u(b):
    return pltpu.bitcast(b, u32)


def _kernel(x_hbm, k_hbm, v_hbm, wq_hbm, wo_hbm, wr_hbm, wg_hbm, wu_hbm, wd_hbm, c_hbm, wmod_hbm,
            out_hbm,
            xo_v, k_v, wq_v, wo_v, wr_v, wg_v, wu_v, wd_v, c_v, wmod_v,
            hce_v, hco_v, o_v, qa_v, qb_v, mod_v, wb_v, wqc_v, acca_v, accb_v, slab_v,
            sx, swq, swm, sw, so, sk, sm):
    x_v = xo_v.at[0]
    h2_v = xo_v.at[1]
    out_v = xo_v.at[2]
    k_u = k_v.bitcast(u32)
    wq_u = wq_v.bitcast(u32)
    wo_u = wo_v.bitcast(u32)
    wg_u = wg_v.bitcast(u32)
    wu_u = wu_v.bitcast(u32)
    wd_u = wd_v.bitcast(u32)
    wmod_u = wmod_v.bitcast(u32)
    hce_u = hce_v.bitcast(u32)
    hco_u = hco_v.bitcast(u32)
    o_u = o_v.bitcast(u32)
    qa_u = qa_v.bitcast(u32)
    qb_u = qb_v.bitcast(u32)
    wb_u = wb_v.bitcast(u32)
    wqc_u = wqc_v.bitcast(u32)

    cp_c = pltpu.make_async_copy(c_hbm, c_v, sm.at[0])
    cp_wr = pltpu.make_async_copy(wr_hbm, wr_v, sm.at[1])
    win = pl.ds(SK - W, W)
    cp_k = [pltpu.make_async_copy(k_hbm.at[g, win, :], k_v.at[g], sk.at[min(g, 1)])
            for g in range(HKV)]
    cp_v = [pltpu.make_async_copy(v_hbm.at[g, win, :], wb_v.at[WB_V, pl.ds(g * W, W), :], sk.at[1])
            for g in range(HKV)]
    cp_vq = [pltpu.make_async_copy(v_hbm.at[g, win, :], wqc_v.at[WQC_V + g], sk.at[1])
             for g in range(HKV)]
    cp_ve = pltpu.make_async_copy(v_hbm.at[0, win, :], hce_v.at[7 * QT], sk.at[0])
    cp_vo = pltpu.make_async_copy(v_hbm.at[0, win, :], hco_v.at[7 * QT], sk.at[0])

    def cp_x(i, sem=None):
        r = pl.ds(pl.multiple_of(i * BM, BM), BM)
        return pltpu.make_async_copy(x_hbm.at[r, :], x_v.at[r, :], sx.at[sem if sem is not None else i])

    def cp_out(i):
        r = pl.ds(pl.multiple_of(i * BM, BM), BM)
        return pltpu.make_async_copy(out_v.at[r, :], out_hbm.at[r, :], so.at[0])

    def cp_tile(w_hbm, w_v, sem, sem_of, n):
        return pltpu.make_async_copy(w_hbm.at[:, pl.ds(n * 128, 128)], w_v.at[n], sem.at[sem_of(n)])

    cp_wq = functools.partial(cp_tile, wq_hbm, wq_v, swq, lambda n: n % NP if n < REP else NP + (n >= 2 * REP))
    cp_wm = functools.partial(cp_tile, wmod_hbm, wmod_v, swm, lambda n: min(n, 2 * NT))
    cp_wo = functools.partial(cp_tile, wo_hbm, wo_v, sw, lambda n: 0)
    cp_wg = functools.partial(cp_tile, wg_hbm, wg_v, sw, lambda n: 1)
    cp_wu = functools.partial(cp_tile, wu_hbm, wu_v, sw, lambda n: 2)
    cp_wd = functools.partial(cp_tile, wd_hbm, wd_v, sw, lambda n: 3)

    cp_c.start()
    cp_x(0).start()
    cp_x(1).start()
    cp_c.wait()
    for n in range(2 * NT):
        cp_wm(n).start()
    cc = c_v[...].astype(f32)
    sc16 = jnp.broadcast_to((cc * jax.nn.sigmoid(cc)).astype(bf16), (16, D))

    def mod_tile(n):
        r = jnp.dot(sc16, _b(wmod_u[n]), preferred_element_type=f32)[0:8]
        r = r.astype(bf16).astype(f32)
        if n // NT in (1, 4):
            r = 1.0 + r
        mod_v[n // NT, :, (n % NT) * 128:(n % NT + 1) * 128] = r

    def store_hc(h, hc_v, r):
        ht, hb = h[:16], h[16:]
        a11, a12, a21, a22 = ht[:, :QH], ht[:, QH:], hb[:, :QH], hb[:, QH:]
        combos = (a11 + a22, a21 + a22, a11, a22, a11 + a12, a21 - a11, a12 - a22)
        for ci, val in enumerate(combos):
            vb = val.astype(bf16)
            for kt in range(QT):
                hc_v[ci * QT + kt, r, :] = vb[:, kt * 128:(kt + 1) * 128]

    def piece_rows(i, c):
        return (pl.ds(pl.multiple_of(i * BM + 16 * c, 16), 16),
                pl.ds(pl.multiple_of(i * BM + HM + 16 * c, 16), 16))

    def ln1_piece(i, hc_v, c):
        rt, rb = piece_rows(i, c)
        x = jnp.concatenate([x_v[rt, :], x_v[rb, :]], axis=0).astype(f32)
        h = _normalize(x) * _rows(mod_v[1], 32) + _rows(mod_v[0], 32)
        store_hc(h, hc_v, pl.ds(pl.multiple_of((i // 2) * HM + 16 * c, 16), 16))

    def normalize_block(i, dst):
        for c in range(HM // 16):
            rt, rb = 16 * c, HM + 16 * c
            x = jnp.concatenate([x_v[i * BM + rt:i * BM + rt + 16, :], x_v[i * BM + rb:i * BM + rb + 16, :]], axis=0)
            dst[32 * c:32 * c + 32, :] = _normalize(x.astype(f32))

    def modulate_block(src, hc_v):
        for c in range(HM // 16):
            h = src[32 * c:32 * c + 32, :] * _rows(mod_v[1], 32) + _rows(mod_v[0], 32)
            store_hc(h, hc_v, pl.ds(16 * c, 16))

    cp_x(0).wait()
    normalize_block(0, acca_v)
    cp_x(1).wait()
    normalize_block(1, accb_v)
    wq_first = [j + NP * hi for j in range(NP) for hi in range(2)]
    for n in range(2 * NT):
        cp_wm(n).wait()
        if n == 11:
            for nn in wq_first:
                cp_wq(nn).start()
            cp_k[0].start()
            cp_ve.start()
            cp_vo.start()
        mod_tile(n)

    def wq_combo(grp):
        pair = grp // 8
        r0 = pl.multiple_of((grp % 8) * 32, 32)
        lo = (pair // NP) * REP + pair % NP
        t0 = pair * 5
        for k in range(4):
            r = pl.ds(pl.multiple_of(r0 + 8 * k, 8), 8)
            r2 = pl.ds(pl.multiple_of(r0 + (QH // 2 + 8 * k), 8), 8)
            b11 = _b(wq_u[lo, r, :]).astype(f32)
            b21 = _b(wq_u[lo, r2, :]).astype(f32)
            b12 = _b(wq_u[lo + NP, r, :]).astype(f32)
            b22 = _b(wq_u[lo + NP, r2, :]).astype(f32)
            for ci, val in enumerate((b11 + b22, b12 - b22, b21 - b11, b11 + b12, b21 + b22)):
                wqc_v[t0 + ci, pl.ds(pl.multiple_of(2 * r0 + 16 * k, 16), 16), :] = val.astype(bf16)

    def wo_combo(grp):
        n = grp // (KH // 64)
        r0 = pl.multiple_of((grp % (KH // 64)) * 32, 32)
        for k in range(4):
            r = pl.ds(pl.multiple_of(r0 + 8 * k, 8), 8)
            r2 = pl.ds(pl.multiple_of(r0 + (KH // 2 + 8 * k), 8), 8)
            b11 = _b(wo_u[n, r, :]).astype(f32)
            b21 = _b(wo_u[n, r2, :]).astype(f32)
            b12 = _b(wo_u[NH + n, r, :]).astype(f32)
            b22 = _b(wo_u[NH + n, r2, :]).astype(f32)
            for ci, val in enumerate((b11 + b22, b12 - b22, b21 - b11, b11 + b12, b21 + b22)):
                wb_v[WB_WO + ci * NH + n, pl.ds(pl.multiple_of(2 * r0 + 16 * k, 16), 16), :] = val.astype(bf16)

    GQ = NP * 8
    NWO = NH * (KH // 64)

    qscale = (DH ** -0.5) * LOG2E

    def qprod(name, g, i, hc_u, jp):
        r = pl.ds(pl.multiple_of((i // 2) * (HM // 2), HM // 2), HM // 2)
        a = jnp.concatenate([_b(hc_u[HC[name] * QT + kt, r, :]) for kt in range(QT)], axis=1)
        if name == "m2":
            b = wq_u[g * REP + jp, 0:QH // 2, :]
        elif name == "m5":
            b = wq_u[g * REP + jp + NP, QH // 2:QH, :]
        else:
            b = wqc_u[(g * NP + jp) * 5 + WC[name]]
        return jnp.dot(a, _b(b), preferred_element_type=f32)

    def qstore(q_dst, j, half, val):
        q_dst[j, half * HM:(half + 1) * HM, :] = (val * qscale).astype(bf16)

    def qproj_part(g, i, hc_u, q_dst, jp, part, carry):
        prod = lambda name: qprod(name, g, i, hc_u, jp)
        if part == 0:
            c22 = prod("m6")
            m3 = prod("m3")
            c22 = c22 + m3
            m5 = prod("m5")
            qstore(q_dst, jp + NP, 0, m3 + m5)
            return prod("m7") - m5, c22
        c11, c22 = carry
        m1 = prod("m1")
        c11 = c11 + m1
        c22 = c22 + m1
        m4 = prod("m4")
        qstore(q_dst, jp, 0, c11 + m4)
        m2 = prod("m2")
        qstore(q_dst, jp, 1, m4 + m2)
        qstore(q_dst, jp + NP, 1, c22 - m2)
        return None

    def kv_rows(g):
        return pl.ds(pl.multiple_of(g * (W // 2), W // 2), W // 2)

    def qk(g, q_src, j):
        return lax.dot_general(_b(q_src[j]), _b(k_u[g]), NT_DIMS, preferred_element_type=f32)

    def softmax_pv(g, i, j, s, v_src):
        m = jnp.max(s, axis=-1, keepdims=True)
        e = jnp.exp2(s - m)
        l = jnp.sum(e, axis=-1, keepdims=True)
        p = (e * (1.0 / l)).astype(bf16)
        o = jnp.dot(p, _b(v_src(g)), preferred_element_type=f32)
        o_v[g * REP + j, pl.ds(pl.multiple_of(i * BM, BM), BM), :] = o.astype(bf16)

    v_wb = lambda g: wb_u[WB_V, kv_rows(g), :]
    v_wq = lambda g: wqc_u[WQC_V + g]
    v_he = lambda g: hce_u[7 * QT]
    v_ho = lambda g: hco_u[7 * QT]

    def step(ga, ia, q_src, v_src, gq=None, iq=None, hc_u=None, q_dst=None, before=None, after=None):
        s = qk(ga, q_src, 0)
        carry = None
        for j in range(REP):
            s_next = qk(ga, q_src, j + 1) if j + 1 < REP else None
            if q_dst is not None:
                carry = qproj_part(gq, iq, hc_u, q_dst, j // 2, j % 2, carry)
            if before is not None:
                before(j)
            softmax_pv(ga, ia, j, s, v_src)
            if after is not None:
                after(j)
            s = s_next

    modulate_block(acca_v, hce_v)
    modulate_block(accb_v, hco_v)
    for jp in range(NP):
        cp_wq(jp).wait()
        cp_wq(jp + NP).wait()
        if jp == 1:
            cp_x(2, 2).start()
            cp_x(3, 2).start()
        for grp in range(jp * 8, (jp + 1) * 8):
            wq_combo(grp)
        carry = qproj_part(0, 0, hce_u, qa_v, jp, 0, None)
        qproj_part(0, 0, hce_u, qa_v, jp, 1, carry)
    for i in range(4, NB):
        cp_x(i, 1 + i // 2).start()
    for n in range(REP, 2 * REP):
        cp_wq(n).start()
    for g in range(1, HKV):
        cp_k[g].start()
    for g in range(HKV):
        cp_v[g].start()
        cp_vq[g].start()
    cp_k[0].wait()
    cp_ve.wait()
    cp_vo.wait()

    def loop1(p, _):
        @pl.when(p == 1)
        def _():
            for n in range(REP, 2 * REP):
                cp_wq(n).wait()
            for n in range(2 * REP, 4 * REP):
                cp_wq(n).start()

        @pl.when(p == 2)
        def _():
            for n in range(NT):
                cp_wo(n).start()
            cp_wr.start()

        @pl.when(p == 3)
        def _():
            for n in range(2 * NT, NMOD):
                cp_wm(n).start()

        @pl.when(p < NB // 2 - 1)
        def _():
            cp_x(2 * p + 2, 2 + p).wait()
            cp_x(2 * p + 3, 2 + p).wait()

        @pl.when(p == 2)
        def _():
            for grp in range(GQ, 2 * GQ):
                wq_combo(grp)

        t = 2 * p
        t2 = t + 2
        ia, ib = jnp.minimum(t + 2, NB - 2), jnp.minimum(t + 3, NB - 1)
        step(0, t, qa_u, v_he, 0, t + 1, hco_u, qb_v, after=lambda j: ln1_piece(ia, hce_v, j))
        step(0, t + 1, qb_u, v_ho, t2 // NB, t2 % NB, hce_u, qa_v, after=lambda j: ln1_piece(ib, hco_v, j))
        return 0

    lax.fori_loop(0, NB // 2, loop1, 0)

    for n in range(2 * REP, 4 * REP):
        cp_wq(n).wait()
    for g in range(1, HKV):
        cp_k[g].wait()
    for g in range(HKV):
        cp_v[g].wait()
        cp_vq[g].wait()
    for n in range(NT):
        cp_wo(n).wait()

    NSTEP = HKV * NB

    def loop2(p, _):
        @pl.when(p == 0)
        def _():
            for n in range(NF):
                cp_wg(n).start()

        @pl.when(p == 1)
        def _():
            for n in range(NF):
                cp_wu(n).start()

        @pl.when(p == 2)
        def _():
            for n in range(NT):
                cp_wd(n).start()

        t = NB + 2 * p
        t1, t2 = t + 1, t + 2
        grp = 2 * GQ + p * 2 * REP
        step(t // NB, t % NB, qa_u, v_wq, t1 // NB, t1 % NB, hco_u, qb_v, after=lambda j: wq_combo(grp + j))
        step(t1 // NB, t1 % NB, qb_u, v_wq, t2 // NB, t2 % NB, hce_u, qa_v,
             after=lambda j: wq_combo(grp + REP + j))
        return 0

    NA = 2 * GQ // (2 * REP)

    lax.fori_loop(0, NA, loop2, 0)

    def loop3(p, _):
        t = NB + 2 * (NA + p)
        t1, t2 = t + 1, t + 2
        grp = p * 2 * REP
        step(t // NB, t % NB, qa_u, v_wb, t1 // NB, t1 % NB, hco_u, qb_v, after=lambda j: wo_combo(grp + j))
        step(t1 // NB, t1 % NB, qb_u, v_wb, t2 // NB, t2 % NB, hce_u, qa_v,
             after=lambda j: wo_combo(grp + REP + j))
        return 0

    NC = (NSTEP - NB) // 2 - 1 - NA
    lax.fori_loop(0, NC, loop3, 0)
    WO_DONE = NC * 2 * REP

    ac_jobs = [(hd, rg) for hd in range(HH) for rg in range(HM // 16)]

    def a_combo(i, slot, jobs):
        for hd, rg in jobs:
            rt = pl.ds(pl.multiple_of(i * HM + rg * 8, 8), 8)
            rb = pl.ds(pl.multiple_of(i * HM + HM // 2 + rg * 8, 8), 8)
            a11 = _b(o_u[hd, rt, :]).astype(f32)
            a12 = _b(o_u[HH + hd, rt, :]).astype(f32)
            a21 = _b(o_u[hd, rb, :]).astype(f32)
            a22 = _b(o_u[HH + hd, rb, :]).astype(f32)
            r = hd * HM + rg * 16
            for ci, val in enumerate((a11 + a22, a21 + a22, a11 + a12, a21 - a11, a12 - a22)):
                wb_v[WB_AC + slot * 5 + ci, r:r + 16, :] = val.astype(bf16)

    cp_wr.wait()
    wr16 = jnp.broadcast_to(wr_v[...].reshape(1, D), (16, D))

    def olhs(kind, i, slot):
        if kind == "m3":
            r = pl.ds(pl.multiple_of(i * HM, HM // 2), HM // 2)
            return jnp.concatenate([_b(o_u[hd, r, :]) for hd in range(HH)], axis=1)
        if kind == "m4":
            r = pl.ds(pl.multiple_of(i * HM + HM // 2, HM // 2), HM // 2)
            return jnp.concatenate([_b(o_u[HH + hd, r, :]) for hd in range(HH)], axis=1)
        return jnp.concatenate(
            [_b(wb_u[WB_AC + slot * 5 + AC[kind], hd * (HM // 2):(hd + 1) * (HM // 2), :]) for hd in range(HH)],
            axis=1)

    def orhs(kind, n):
        if kind == "m2":
            return _b(wo_u[n, 0:KH // 2, :])
        if kind == "m5":
            return _b(wo_u[NH + n, KH // 2:KH, :])
        return _b(wb_u[WB_WO + WC[kind] * NH + n])

    def oprod(kind, i, slot, n):
        return jnp.dot(olhs(kind, i, slot), orhs(kind, n), preferred_element_type=f32)

    def epilogue(i, acc_r, c0, nc, sub):
        hs = []
        for o in range(0, nc, sub):
            r = pl.ds(pl.multiple_of(i * BM + c0 + o, sub), sub)
            x1 = x_v[r, :].astype(f32) + _rows(mod_v[2], sub) * acc_r[c0 + o:c0 + o + sub, :]
            h2 = _normalize(x1) * _rows(mod_v[4], sub) + _rows(mod_v[3], sub)
            h2b = h2.astype(bf16)
            h2_v[r, :] = h2b
            out_v[r, :] = (x1 + _rows(mod_v[5], sub) * h2).astype(bf16)
            hs.append(h2b)
        h2b = jnp.concatenate(hs, axis=0) if len(hs) > 1 else hs[0]
        score = lax.dot_general(wr16, h2b, NT_DIMS, preferred_element_type=f32)
        return score[0:8, :].astype(bf16).astype(f32)

    def update_best(state, i, scores):
        best_v, best_i = state
        r = jnp.concatenate(scores, axis=1)
        rows = i * BM + lax.broadcasted_iota(jnp.int32, (8, BM), 1)
        better = r > best_v
        return jnp.where(better, r, best_v), jnp.where(better, rows, best_i)

    def block_steps(i, slot, acc_w, i_prev, acc_r, result, inext=None, snext=None, do_epi=True):
        scores = []
        nprod = NH * 7
        per = len(ac_jobs) // nprod
        extra = len(ac_jobs) - per * nprod
        pos = [0, 0]

        def fill():
            cnt = per + (1 if pos[1] < extra else 0)
            if inext is not None:
                a_combo(inext, snext, ac_jobs[pos[0]:pos[0] + cnt])
            pos[0] += cnt
            pos[1] += 1

        def prod(kind, n):
            val = oprod(kind, i, slot, n)
            fill()
            return val

        def fill_only():
            fill()

        for n in range(NH):
            cl = slice(n * 128, (n + 1) * 128)
            cr = slice((NH + n) * 128, (NH + n + 1) * 128)
            c22 = prod("m6", n)
            yield
            m3 = prod("m3", n)
            yield
            c22 = c22 + m3
            m5 = prod("m5", n)
            yield
            acc_w[0:HM, cr] = m3 + m5
            c11 = prod("m7", n) - m5
            yield
            m1 = prod("m1", n)
            yield
            c11 = c11 + m1
            c22 = c22 + m1
            m4 = prod("m4", n)
            yield
            acc_w[0:HM, cl] = c11 + m4
            m2 = prod("m2", n)
            acc_w[HM:BM, cl] = m4 + m2
            acc_w[HM:BM, cr] = c22 - m2
            if do_epi and n in (1, 3):
                scores.append(epilogue(i_prev, acc_r, (n // 2) * HM, HM, SUB))
            if n < NH - 1:
                yield
        if do_epi:
            result[0] = update_best(result[0], i_prev, scores)
            cp_out(i_prev).start()

    def block(i, slot, acc_w, i_prev, acc_r, state, inext=None, snext=None):
        result = [state]
        for _ in block_steps(i, slot, acc_w, i_prev, acc_r, result, inext, snext):
            pass
        return result[0]

    for n in range(2 * NT, NMOD):
        cp_wm(n).wait()
    step(HKV - 1, NB - 2, qa_u, v_wb, HKV - 1, NB - 1, hco_u, qb_v,
         after=lambda j: (wo_combo(WO_DONE + 2 * j), wo_combo(WO_DONE + 2 * j + 1),
                          a_combo(0, 0, ac_jobs[j * 16:(j + 1) * 16])))

    first = block_steps(0, 0, acca_v, None, None, None, 1, 1, do_epi=False)

    def first_fill(j):
        for n in range(2 * NT + 4 * j, 2 * NT + 4 * j + 4):
            mod_tile(n)
        for _ in range(4 if j % 2 else 3):
            next(first, None)

    step(HKV - 1, NB - 1, qb_u, v_wb, before=first_fill)
    for _ in first:
        pass

    state = (jnp.full((8, BM), -jnp.inf, f32), jnp.zeros((8, BM), jnp.int32))

    def loopb(p, state):
        i = 2 * p
        state = block(i + 1, 1, accb_v, i, acca_v, state, i + 2, 0)
        state = block(i + 2, 0, acca_v, i + 1, accb_v, state, i + 3, 1)
        return state

    state = lax.fori_loop(0, NB // 2 - 1, loopb, state)
    for n in range(NF):
        cp_wg(n).wait()
        cp_wu(n).wait()
    for n in range(NT):
        cp_wd(n).wait()
    state = block(NB - 1, 1, accb_v, NB - 2, acca_v, state)
    scores = [epilogue(NB - 1, accb_v, c * 128, 128, 64) for c in range(BM // 128)]
    best_v, best_i = update_best(state, NB - 1, scores)
    cp_out(NB - 1).start()

    rmax = jnp.max(best_v, axis=1, keepdims=True)
    idx = jnp.min(jnp.where(best_v == rmax, best_i, S), axis=1, keepdims=True)
    base = pl.multiple_of((idx[0, 0] // 16) * 16, 16)
    hs = h2_v[pl.ds(base, 16), :]
    acts = []
    for n in range(NF):
        gate = jnp.dot(hs, _b(wg_u[n]), preferred_element_type=f32).astype(bf16).astype(f32)
        up = jnp.dot(hs, _b(wu_u[n]), preferred_element_type=f32).astype(bf16).astype(f32)
        acts.append(((gate * jax.nn.sigmoid(gate)).astype(bf16).astype(f32) * up).astype(bf16))
    act = jnp.concatenate(acts, axis=1)
    old = out_v[pl.ds(base, 16), :].astype(f32)
    sel = base + lax.broadcasted_iota(jnp.int32, (16, 1), 0) == idx[0:1, :]
    weight = jax.nn.sigmoid(rmax[0:1, :])
    for n in range(NT):
        cols = slice(n * 128, (n + 1) * 128)
        y = jnp.dot(act, _b(wd_u[n]), preferred_element_type=f32).astype(bf16).astype(f32)
        new = old[:, cols] + _rows(mod_v[5, :, cols], 16) * (y * weight)
        slab_v[:, cols] = jnp.where(sel, new, old[:, cols]).astype(bf16)
    for i in range(NB):
        cp_out(i).wait()
    cp_slab = pltpu.make_async_copy(slab_v, out_hbm.at[pl.ds(base, 16), :], sm.at[2])
    cp_slab.start()
    cp_slab.wait()


@jax.jit
def pallas_adaLN_cond__sliding_block_cached__moe_arch_mod__prompt_kernel(
        A_x, A_k_cache, A_v_cache, A_wq, A_wo, B_x, B_w_r, B_w_gate, B_w_up, B_w_down, c, w_mod):
    x = A_x.reshape(S, D)
    k = A_k_cache.reshape(HKV, SK, DH)
    v = A_v_cache.reshape(HKV, SK, DH)
    wr = B_w_r
    anyspec = pl.BlockSpec(memory_space=pl.ANY)
    dma = pltpu.SemaphoreType.DMA
    out = pl.pallas_call(
        _kernel,
        out_shape=jax.ShapeDtypeStruct((S, D), bf16),
        in_specs=[anyspec] * 11,
        out_specs=anyspec,
        scratch_shapes=[
            pltpu.VMEM((3, S, D), bf16),
            pltpu.VMEM((HKV, W, DH), bf16),
            pltpu.VMEM((HQ, D, 128), bf16),
            pltpu.VMEM((NT, HQ * DH, 128), bf16),
            pltpu.VMEM((D,), bf16),
            pltpu.VMEM((NF, D, 128), bf16),
            pltpu.VMEM((NF, D, 128), bf16),
            pltpu.VMEM((NT, F, 128), bf16),
            pltpu.VMEM((1, D), bf16),
            pltpu.VMEM((NMOD, D, 128), bf16),
            pltpu.VMEM((7 * QT + 1, S // 4, 128), bf16),
            pltpu.VMEM((7 * QT + 1, S // 4, 128), bf16),
            pltpu.VMEM((HQ, S, 128), bf16),
            pltpu.VMEM((REP, BM, 128), bf16),
            pltpu.VMEM((REP, BM, 128), bf16),
            pltpu.VMEM((6, 8, D), f32),
            pltpu.VMEM((WB_SLOTS, KH, 128), bf16),
            pltpu.VMEM((WQC_V + HKV, QH, 128), bf16),
            pltpu.VMEM((BM, D), f32),
            pltpu.VMEM((BM, D), f32),
            pltpu.VMEM((16, D), bf16),
            dma((1 + NB // 2,)), dma((NP + 2,)), dma((2 * NT + 1,)), dma((4,)), dma((1,)), dma((2,)), dma((3,)),
        ],
        compiler_params=pltpu.CompilerParams(vmem_limit_bytes=124 * 1024 * 1024),
    )(x, k, v, A_wq, A_wo, wr, B_w_gate, B_w_up, B_w_down, c, w_mod)
    return out.reshape(1, S, D)
```

```python
import functools

import jax
import jax.numpy as jnp
from jax import lax
import jax.experimental.pallas as pl
import jax.experimental.pallas.tpu as pltpu

S, D = 2048, 1024
HQ, HKV, DH = 32, 4, 128
SK = 2048
W = 512
REP = HQ // HKV
F = 3584
EPS = 1e-5
QSCALE = DH ** -0.5 * 1.4426950408889634
BM = 256
NB = S // BM
HM = BM // 2
NT = D // 128
NF = F // 128
NMOD = 6 * NT
SUB = 16
KH = HQ * DH // 2
NH = NT // 2
HH = HQ // 2
QH = D // 2
QT = QH // 128
NP = REP // 2
WB_WO, WB_AC, WB_V, WB_WQ = 0, 20, 30, 31
WB_SLOTS = 51
HC = {"m1": 0, "m2": 1, "m3": 2, "m4": 3, "m5": 4, "m6": 5, "m7": 6}
WC = {"m1": 0, "m3": 1, "m4": 2, "m6": 3, "m7": 4}
AC = {"m1": 0, "m2": 1, "m5": 2, "m6": 3, "m7": 4}

f32 = jnp.float32
bf16 = jnp.bfloat16
u32 = jnp.uint32
NT_DIMS = (((1,), (1,)), ((), ()))


def _rows(m8, n):
    return jnp.concatenate([m8] * (n // 8), axis=0) if n > 8 else m8


def _hint(x, m):
    return x if isinstance(x, int) else pl.multiple_of(x, m)


def _normalize(x):
    xc = x - jnp.mean(x, axis=-1, keepdims=True)
    return xc * lax.rsqrt(jnp.mean(xc * xc, axis=-1, keepdims=True) + EPS)


def _b(u):
    return pltpu.bitcast(u, bf16)


def _kernel(x_hbm, k_hbm, v_hbm, wq_hbm, wo_hbm, wr_hbm, wg_hbm, wu_hbm, wd_hbm, c_hbm, wmod_hbm,
            out_hbm,
            xo_v, k_v, ws_v, wr_v, wg_v, wu_v, wd_v, c_v, wmod_v,
            hce_v, hco_v, o_v, qa_v, qb_v, mod_v, wb_v, acca_v, accb_v, slab_v,
            sx, swq, swm, sw, so, sk, sm):
    x_v = xo_v.at[0]
    h2_v = xo_v.at[1]
    out_v = xo_v.at[2]
    k_u = k_v.bitcast(u32)
    ws_u = ws_v.bitcast(u32)
    wg_u = wg_v.bitcast(u32)
    wu_u = wu_v.bitcast(u32)
    wd_u = wd_v.bitcast(u32)
    wmod_u = wmod_v.bitcast(u32)
    hce_u = hce_v.bitcast(u32)
    hco_u = hco_v.bitcast(u32)
    o_u = o_v.bitcast(u32)
    qa_u = qa_v.bitcast(u32)
    qb_u = qb_v.bitcast(u32)
    wb_u = wb_v.bitcast(u32)

    cp_c = pltpu.make_async_copy(c_hbm, c_v, sm.at[0])
    cp_wr = pltpu.make_async_copy(wr_hbm, wr_v, sm.at[1])
    win = pl.ds(SK - W, W)
    cp_k = [pltpu.make_async_copy(k_hbm.at[g, win, :], k_v.at[g], sk.at[min(g, 1)])
            for g in range(HKV)]
    cp_v = [pltpu.make_async_copy(v_hbm.at[g, win, :], wb_v.at[WB_V, pl.ds(g * W, W), :], sk.at[1])
            for g in range(HKV)]
    cp_ve = pltpu.make_async_copy(v_hbm.at[0, win, :], hce_v.at[7 * QT], sk.at[0])
    cp_vo = pltpu.make_async_copy(v_hbm.at[0, win, :], hco_v.at[7 * QT], sk.at[0])

    def cp_x(i, sem=None):
        r = pl.ds(pl.multiple_of(i * BM, BM), BM)
        return pltpu.make_async_copy(x_hbm.at[r, :], x_v.at[r, :], sx.at[sem if sem is not None else i])

    def cp_out(i):
        r = pl.ds(pl.multiple_of(i * BM, BM), BM)
        return pltpu.make_async_copy(out_v.at[r, :], out_hbm.at[r, :], so.at[0])

    def cp_tile(w_hbm, w_v, sem, sem_of, n):
        return pltpu.make_async_copy(w_hbm.at[:, pl.ds(n * 128, 128)], w_v.at[n], sem.at[sem_of(n)])


    def cp_wq(n):
        return pltpu.make_async_copy(wq_hbm.at[:, pl.ds(n * 128, 128)], ws_v.at[n // 4, pl.ds((n % 4) * D, D), :],
                                     swq.at[n % NP if n < REP else NP + (n >= 2 * REP)])

    def cp_wo(n):
        return pltpu.make_async_copy(wo_hbm.at[:, pl.ds(n * 128, 128)], ws_v.at[NT + n], sw.at[0])

    cp_wm = functools.partial(cp_tile, wmod_hbm, wmod_v, swm, lambda n: min(n, 2 * NT))
    cp_wg = functools.partial(cp_tile, wg_hbm, wg_v, sw, lambda n: 1)
    cp_wu = functools.partial(cp_tile, wu_hbm, wu_v, sw, lambda n: 2)
    cp_wd = functools.partial(cp_tile, wd_hbm, wd_v, sw, lambda n: 3)

    cp_c.start()
    cp_x(0).start()
    cp_x(1).start()
    cp_c.wait()
    for n in range(2 * NT):
        cp_wm(n).start()
    cc = c_v[...].astype(f32)
    sc16 = jnp.broadcast_to((cc * jax.nn.sigmoid(cc)).astype(bf16), (16, D))

    def mod_tile(n):
        r = jnp.dot(sc16, _b(wmod_u[n]), preferred_element_type=f32)[0:8]
        r = r.astype(bf16).astype(f32)
        if n // NT in (1, 4):
            r = 1.0 + r
        if n // NT < 2:
            r = r * QSCALE
        mod_v[n // NT, :, (n % NT) * 128:(n % NT + 1) * 128] = r

    def store_hc(h, hc_v, r):
        ht, hb = h[:16], h[16:]
        a11, a12, a21, a22 = ht[:, :QH], ht[:, QH:], hb[:, :QH], hb[:, QH:]
        combos = (a11 + a22, a21 + a22, a11, a22, a11 + a12, a21 - a11, a12 - a22)
        for ci, val in enumerate(combos):
            vb = val.astype(bf16)
            for kt in range(QT):
                hc_v[ci * QT + kt, r, :] = vb[:, kt * 128:(kt + 1) * 128]

    def piece_rows(i, c):
        return (pl.ds(pl.multiple_of(i * BM + 16 * c, 16), 16),
                pl.ds(pl.multiple_of(i * BM + HM + 16 * c, 16), 16))

    def ln1_piece(i, hc_v, c):
        rt, rb = piece_rows(i, c)
        x = jnp.concatenate([x_v[rt, :], x_v[rb, :]], axis=0).astype(f32)
        h = _normalize(x) * _rows(mod_v[1], 32) + _rows(mod_v[0], 32)
        store_hc(h, hc_v, pl.ds(pl.multiple_of((i // 2) * HM + 16 * c, 16), 16))

    def normalize_block(i, dst):
        for c in range(HM // 16):
            rt, rb = 16 * c, HM + 16 * c
            x = jnp.concatenate([x_v[i * BM + rt:i * BM + rt + 16, :], x_v[i * BM + rb:i * BM + rb + 16, :]], axis=0)
            dst[32 * c:32 * c + 32, :] = _normalize(x.astype(f32))

    def modulate_block(src, hc_v):
        for c in range(HM // 16):
            h = src[32 * c:32 * c + 32, :] * _rows(mod_v[1], 32) + _rows(mod_v[0], 32)
            store_hc(h, hc_v, pl.ds(16 * c, 16))

    cp_x(0).wait()
    normalize_block(0, acca_v)
    cp_x(1).wait()
    normalize_block(1, accb_v)
    wq_first = [j + NP * hi for j in range(NP) for hi in range(2)]
    for n in range(2 * NT):
        cp_wm(n).wait()
        if n == 11:
            for nn in wq_first:
                cp_wq(nn).start()
            cp_k[0].start()
            cp_ve.start()
            cp_vo.start()
        mod_tile(n)

    def combo(job):
        if isinstance(job, int):
            pick = lambda a, b: a if job < 128 else b
            hint = lambda x, m: x
        else:
            is_q = job < 128
            pick = lambda a, b: jnp.where(is_q, a, b)
            hint = pl.multiple_of
        pair, grp_o = job // 8, job - 128
        lo = (pair // NP) * REP + pair % NP
        n = grp_o // 32
        r0 = hint(pick(job % 8, grp_o % 32) * 32, 32)
        half = pick(QH // 2, KH // 2)
        s1, base1 = pick(lo // 4, NT + n), pick((lo % 4) * (D // 2), 0)
        s2, base2 = pick((lo + NP) // 4, NT + NH + n), pick(((lo + NP) % 4) * (D // 2), 0)
        for k in range(4):
            r1 = hint(base1 + r0 + 8 * k, 8)
            r2 = hint(base2 + r0 + 8 * k, 8)
            b11 = _b(ws_u[s1, pl.ds(r1, 8), :]).astype(f32)
            b21 = _b(ws_u[s1, pl.ds(hint(r1 + half, 8), 8), :]).astype(f32)
            b12 = _b(ws_u[s2, pl.ds(r2, 8), :]).astype(f32)
            b22 = _b(ws_u[s2, pl.ds(hint(r2 + half, 8), 8), :]).astype(f32)
            for ci, val in enumerate((b11 + b22, b12 - b22, b21 - b11, b11 + b12, b21 + b22)):
                t = pair * 5 + ci
                slot = pick(WB_WQ + t // 4, WB_WO + ci * NH + n)
                row = hint(pick((t % 4) * QH, 0) + 2 * r0 + 16 * k, 16)
                wb_v[slot, pl.ds(row, 16), :] = val.astype(bf16)

    GQ = NP * 8

    def qprod(name, g, i, hc_u, jp):
        r = pl.ds(pl.multiple_of((i // 2) * (HM // 2), HM // 2), HM // 2)
        a = jnp.concatenate([_b(hc_u[HC[name] * QT + kt, r, :]) for kt in range(QT)], axis=1)
        if name == "m2":
            b = ws_u[2 * g, jp * (D // 2):jp * (D // 2) + QH // 2, :]
        elif name == "m5":
            b = ws_u[2 * g + 1, jp * (D // 2) + QH // 2:(jp + 1) * (D // 2), :]
        else:
            t = (g * NP + jp) * 5 + WC[name]
            b = wb_u[WB_WQ + t // 4, pl.ds(_hint((t % 4) * (QH // 2), QH // 2), QH // 2), :]
        return jnp.dot(a, _b(b), preferred_element_type=f32)

    def qstore(q_dst, j, half, val):
        q_dst[j, half * HM:(half + 1) * HM, :] = val.astype(bf16)

    def qproj_part(g, i, hc_u, q_dst, jp, part, carry):
        prod = lambda name: qprod(name, g, i, hc_u, jp)
        if part == 0:
            c22 = prod("m6")
            m3 = prod("m3")
            c22 = c22 + m3
            m5 = prod("m5")
            qstore(q_dst, jp + NP, 0, m3 + m5)
            return prod("m7") - m5, c22
        c11, c22 = carry
        m1 = prod("m1")
        c11 = c11 + m1
        c22 = c22 + m1
        m4 = prod("m4")
        qstore(q_dst, jp, 0, c11 + m4)
        m2 = prod("m2")
        qstore(q_dst, jp, 1, m4 + m2)
        qstore(q_dst, jp + NP, 1, c22 - m2)
        return None

    def kv_rows(g):
        return pl.ds(pl.multiple_of(g * (W // 2), W // 2), W // 2)

    def qk(g, q_src, j):
        return lax.dot_general(_b(q_src[j]), _b(k_u[g]), NT_DIMS, preferred_element_type=f32)

    def softmax_pv(g, i, j, s, v_src):
        m = jnp.max(s, axis=-1, keepdims=True)
        e = jnp.exp2(s - m)
        l = jnp.sum(e, axis=-1, keepdims=True)
        inv = pl.reciprocal(l, approx=True)
        inv = inv * (2.0 - l * inv)
        p = (e * inv).astype(bf16)
        o = jnp.dot(p, _b(v_src(g)), preferred_element_type=f32)
        o_v[g * REP + j, pl.ds(pl.multiple_of(i * BM, BM), BM), :] = o.astype(bf16)

    v_wb = lambda g: wb_u[WB_V, kv_rows(g), :]
    v_he = lambda g: hce_u[7 * QT]
    v_ho = lambda g: hco_u[7 * QT]

    def step(ga, ia, q_src, v_src, gq=None, iq=None, hc_u=None, q_dst=None, before=None, after=None):
        s = qk(ga, q_src, 0)
        carry = None
        for j in range(REP):
            s_next = qk(ga, q_src, j + 1) if j + 1 < REP else None
            if q_dst is not None:
                carry = qproj_part(gq, iq, hc_u, q_dst, j // 2, j % 2, carry)
            if before is not None:
                before(j)
            softmax_pv(ga, ia, j, s, v_src)
            if after is not None:
                after(j)
            s = s_next

    modulate_block(acca_v, hce_v)
    modulate_block(accb_v, hco_v)
    for jp in range(NP):
        cp_wq(jp).wait()
        cp_wq(jp + NP).wait()
        if jp == 1:
            cp_x(2, 2).start()
            cp_x(3, 2).start()
        for grp in range(jp * 8, (jp + 1) * 8):
            combo(grp)
        carry = qproj_part(0, 0, hce_u, qa_v, jp, 0, None)
        qproj_part(0, 0, hce_u, qa_v, jp, 1, carry)
    for i in range(4, NB):
        cp_x(i, 1 + i // 2).start()
    for n in range(REP, 2 * REP):
        cp_wq(n).start()
    for g in range(1, HKV):
        cp_k[g].start()
    for g in range(HKV):
        cp_v[g].start()
    cp_k[0].wait()
    cp_ve.wait()
    cp_vo.wait()

    def loop1(p, _):
        @pl.when(p == 1)
        def _():
            for n in range(REP, 2 * REP):
                cp_wq(n).wait()
            for n in range(2 * REP, 4 * REP):
                cp_wq(n).start()

        @pl.when(p == 2)
        def _():
            for n in range(NT):
                cp_wo(n).start()
            cp_wr.start()

        @pl.when(p == 3)
        def _():
            for n in range(2 * NT, NMOD):
                cp_wm(n).start()

        @pl.when(p < NB // 2 - 1)
        def _():
            cp_x(2 * p + 2, 2 + p).wait()
            cp_x(2 * p + 3, 2 + p).wait()

        @pl.when(p == 2)
        def _():
            for grp in range(GQ, 2 * GQ):
                combo(grp)

        t = 2 * p
        t2 = t + 2
        ia, ib = jnp.minimum(t + 2, NB - 2), jnp.minimum(t + 3, NB - 1)
        step(0, t, qa_u, v_he, 0, t + 1, hco_u, qb_v, after=lambda j: ln1_piece(ia, hce_v, j))
        step(0, t + 1, qb_u, v_ho, t2 // NB, t2 % NB, hce_u, qa_v, after=lambda j: ln1_piece(ib, hco_v, j))
        return 0

    lax.fori_loop(0, NB // 2, loop1, 0)

    for n in range(2 * REP, 4 * REP):
        cp_wq(n).wait()
    for g in range(1, HKV):
        cp_k[g].wait()
    for g in range(HKV):
        cp_v[g].wait()
    for n in range(NT):
        cp_wo(n).wait()

    NSTEP = HKV * NB

    def loop2(p, _):
        @pl.when(p == 0)
        def _():
            for n in range(NF):
                cp_wg(n).start()

        @pl.when(p == 1)
        def _():
            for n in range(NF):
                cp_wu(n).start()

        @pl.when(p == 2)
        def _():
            for n in range(NT):
                cp_wd(n).start()

        t = NB + 2 * p
        t1, t2 = t + 1, t + 2
        job = 2 * GQ + p * 2 * REP
        step(t // NB, t % NB, qa_u, v_wb, t1 // NB, t1 % NB, hco_u, qb_v, after=lambda j: combo(job + j))
        step(t1 // NB, t1 % NB, qb_u, v_wb, t2 // NB, t2 % NB, hce_u, qa_v, after=lambda j: combo(job + REP + j))
        return 0

    NC = (NSTEP - NB) // 2 - 1
    lax.fori_loop(0, NC, loop2, 0)
    JOBS_DONE = 2 * GQ + NC * 2 * REP

    ac_jobs = [(hd, rg) for hd in range(HH) for rg in range(HM // 16)]

    def a_combo(i, slot, jobs):
        for hd, rg in jobs:
            rt = pl.ds(pl.multiple_of(i * HM + rg * 8, 8), 8)
            rb = pl.ds(pl.multiple_of(i * HM + HM // 2 + rg * 8, 8), 8)
            a11 = _b(o_u[hd, rt, :]).astype(f32)
            a12 = _b(o_u[HH + hd, rt, :]).astype(f32)
            a21 = _b(o_u[hd, rb, :]).astype(f32)
            a22 = _b(o_u[HH + hd, rb, :]).astype(f32)
            r = hd * HM + rg * 16
            for ci, val in enumerate((a11 + a22, a21 + a22, a11 + a12, a21 - a11, a12 - a22)):
                wb_v[WB_AC + slot * 5 + ci, r:r + 16, :] = val.astype(bf16)

    cp_wr.wait()
    wr16 = jnp.broadcast_to(wr_v[...].reshape(1, D), (16, D))

    def olhs(kind, i, slot):
        if kind == "m3":
            r = pl.ds(pl.multiple_of(i * HM, HM // 2), HM // 2)
            return jnp.concatenate([_b(o_u[hd, r, :]) for hd in range(HH)], axis=1)
        if kind == "m4":
            r = pl.ds(pl.multiple_of(i * HM + HM // 2, HM // 2), HM // 2)
            return jnp.concatenate([_b(o_u[HH + hd, r, :]) for hd in range(HH)], axis=1)
        return jnp.concatenate(
            [_b(wb_u[WB_AC + slot * 5 + AC[kind], hd * (HM // 2):(hd + 1) * (HM // 2), :]) for hd in range(HH)],
            axis=1)

    def orhs(kind, n):
        if kind == "m2":
            return _b(ws_u[NT + n, 0:KH // 2, :])
        if kind == "m5":
            return _b(ws_u[NT + NH + n, KH // 2:KH, :])
        return _b(wb_u[WB_WO + WC[kind] * NH + n])

    def oprod(kind, i, slot, n):
        return jnp.dot(olhs(kind, i, slot), orhs(kind, n), preferred_element_type=f32)

    def epilogue(i, acc_r, c0, nc, sub):
        hs = []
        for o in range(0, nc, sub):
            r = pl.ds(pl.multiple_of(i * BM + c0 + o, sub), sub)
            x1 = x_v[r, :].astype(f32) + _rows(mod_v[2], sub) * acc_r[c0 + o:c0 + o + sub, :]
            h2 = _normalize(x1) * _rows(mod_v[4], sub) + _rows(mod_v[3], sub)
            h2b = h2.astype(bf16)
            h2_v[r, :] = h2b
            out_v[r, :] = (x1 + _rows(mod_v[5], sub) * h2).astype(bf16)
            hs.append(h2b)
        h2b = jnp.concatenate(hs, axis=0) if len(hs) > 1 else hs[0]
        score = lax.dot_general(wr16, h2b, NT_DIMS, preferred_element_type=f32)
        return score[0:8, :].astype(bf16).astype(f32)

    def update_best(state, i, scores):
        best_v, best_i = state
        r = jnp.concatenate(scores, axis=1)
        rows = i * BM + lax.broadcasted_iota(jnp.int32, (8, BM), 1)
        better = r > best_v
        return jnp.where(better, r, best_v), jnp.where(better, rows, best_i)

    def block_steps(i, slot, acc_w, i_prev, acc_r, result, inext=None, snext=None, do_epi=True):
        scores = []
        nprod = NH * 7
        per = len(ac_jobs) // nprod
        extra = len(ac_jobs) - per * nprod
        pos = [0, 0]

        def fill():
            cnt = per + (1 if pos[1] < extra else 0)
            if inext is not None:
                a_combo(inext, snext, ac_jobs[pos[0]:pos[0] + cnt])
            pos[0] += cnt
            pos[1] += 1

        def prod(kind, n):
            val = oprod(kind, i, slot, n)
            fill()
            return val

        for n in range(NH):
            cl = slice(n * 128, (n + 1) * 128)
            cr = slice((NH + n) * 128, (NH + n + 1) * 128)
            c22 = prod("m6", n)
            yield
            m3 = prod("m3", n)
            yield
            c22 = c22 + m3
            m5 = prod("m5", n)
            yield
            acc_w[0:HM, cr] = m3 + m5
            c11 = prod("m7", n) - m5
            yield
            m1 = prod("m1", n)
            yield
            c11 = c11 + m1
            c22 = c22 + m1
            m4 = prod("m4", n)
            yield
            acc_w[0:HM, cl] = c11 + m4
            m2 = prod("m2", n)
            acc_w[HM:BM, cl] = m4 + m2
            acc_w[HM:BM, cr] = c22 - m2
            if do_epi and n in (1, 3):
                scores.append(epilogue(i_prev, acc_r, (n // 2) * HM, HM, SUB))
            if n < NH - 1:
                yield
        if do_epi:
            result[0] = update_best(result[0], i_prev, scores)
            cp_out(i_prev).start()

    def block(i, slot, acc_w, i_prev, acc_r, state, inext=None, snext=None):
        result = [state]
        for _ in block_steps(i, slot, acc_w, i_prev, acc_r, result, inext, snext):
            pass
        return result[0]

    for n in range(2 * NT, NMOD):
        cp_wm(n).wait()
    step(HKV - 1, NB - 2, qa_u, v_wb, HKV - 1, NB - 1, hco_u, qb_v,
         after=lambda j: (combo(JOBS_DONE + 2 * j), combo(JOBS_DONE + 2 * j + 1),
                          a_combo(0, 0, ac_jobs[j * 16:(j + 1) * 16])))

    first = block_steps(0, 0, acca_v, None, None, None, 1, 1, do_epi=False)

    def first_fill(j):
        for n in range(2 * NT + 4 * j, 2 * NT + 4 * j + 4):
            mod_tile(n)
        for _ in range(4 if j % 2 else 3):
            next(first, None)

    step(HKV - 1, NB - 1, qb_u, v_wb, before=first_fill)
    for _ in first:
        pass

    state = (jnp.full((8, BM), -jnp.inf, f32), jnp.zeros((8, BM), jnp.int32))

    def loopb(p, state):
        i = 2 * p
        state = block(i + 1, 1, accb_v, i, acca_v, state, i + 2, 0)
        state = block(i + 2, 0, acca_v, i + 1, accb_v, state, i + 3, 1)
        return state

    state = lax.fori_loop(0, NB // 2 - 1, loopb, state)
    for n in range(NF):
        cp_wg(n).wait()
        cp_wu(n).wait()
    for n in range(NT):
        cp_wd(n).wait()
    state = block(NB - 1, 1, accb_v, NB - 2, acca_v, state)
    scores = [epilogue(NB - 1, accb_v, c * 128, 128, 64) for c in range(BM // 128)]
    best_v, best_i = update_best(state, NB - 1, scores)
    cp_out(NB - 1).start()

    rmax = jnp.max(best_v, axis=1, keepdims=True)
    idx = jnp.min(jnp.where(best_v == rmax, best_i, S), axis=1, keepdims=True)
    base = pl.multiple_of((idx[0, 0] // 16) * 16, 16)
    hs = h2_v[pl.ds(base, 16), :]
    acts = []
    for n in range(NF):
        gate = jnp.dot(hs, _b(wg_u[n]), preferred_element_type=f32).astype(bf16).astype(f32)
        up = jnp.dot(hs, _b(wu_u[n]), preferred_element_type=f32).astype(bf16).astype(f32)
        acts.append(((gate * jax.nn.sigmoid(gate)).astype(bf16).astype(f32) * up).astype(bf16))
    act = jnp.concatenate(acts, axis=1)
    old = out_v[pl.ds(base, 16), :].astype(f32)
    sel = base + lax.broadcasted_iota(jnp.int32, (16, 1), 0) == idx[0:1, :]
    weight = jax.nn.sigmoid(rmax[0:1, :])
    for n in range(NT):
        cols = slice(n * 128, (n + 1) * 128)
        y = jnp.dot(act, _b(wd_u[n]), preferred_element_type=f32).astype(bf16).astype(f32)
        new = old[:, cols] + _rows(mod_v[5, :, cols], 16) * (y * weight)
        slab_v[:, cols] = jnp.where(sel, new, old[:, cols]).astype(bf16)
    for i in range(NB):
        cp_out(i).wait()
    cp_slab = pltpu.make_async_copy(slab_v, out_hbm.at[pl.ds(base, 16), :], sm.at[2])
    cp_slab.start()
    cp_slab.wait()


@jax.jit
def pallas_adaLN_cond__sliding_block_cached__moe_arch_mod__prompt_kernel(
        A_x, A_k_cache, A_v_cache, A_wq, A_wo, B_x, B_w_r, B_w_gate, B_w_up, B_w_down, c, w_mod):
    x = A_x.reshape(S, D)
    k = A_k_cache.reshape(HKV, SK, DH)
    v = A_v_cache.reshape(HKV, SK, DH)
    wr = B_w_r
    anyspec = pl.BlockSpec(memory_space=pl.ANY)
    dma = pltpu.SemaphoreType.DMA
    out = pl.pallas_call(
        _kernel,
        out_shape=jax.ShapeDtypeStruct((S, D), bf16),
        in_specs=[anyspec] * 11,
        out_specs=anyspec,
        scratch_shapes=[
            pltpu.VMEM((3, S, D), bf16),
            pltpu.VMEM((HKV, W, DH), bf16),
            pltpu.VMEM((2 * NT, HQ * DH, 128), bf16),
            pltpu.VMEM((D,), bf16),
            pltpu.VMEM((NF, D, 128), bf16),
            pltpu.VMEM((NF, D, 128), bf16),
            pltpu.VMEM((NT, F, 128), bf16),
            pltpu.VMEM((1, D), bf16),
            pltpu.VMEM((NMOD, D, 128), bf16),
            pltpu.VMEM((7 * QT + 1, S // 4, 128), bf16),
            pltpu.VMEM((7 * QT + 1, S // 4, 128), bf16),
            pltpu.VMEM((HQ, S, 128), bf16),
            pltpu.VMEM((REP, BM, 128), bf16),
            pltpu.VMEM((REP, BM, 128), bf16),
            pltpu.VMEM((6, 8, D), f32),
            pltpu.VMEM((WB_SLOTS, KH, 128), bf16),
            pltpu.VMEM((BM, D), f32),
            pltpu.VMEM((BM, D), f32),
            pltpu.VMEM((16, D), bf16),
            dma((1 + NB // 2,)), dma((NP + 2,)), dma((2 * NT + 1,)), dma((4,)), dma((1,)), dma((2,)), dma((3,)),
        ],
        compiler_params=pltpu.CompilerParams(vmem_limit_bytes=124 * 1024 * 1024),
    )(x, k, v, A_wq, A_wo, wr, B_w_gate, B_w_up, B_w_down, c, w_mod)
    return out.reshape(1, S, D)
```

```python
import functools

import jax
import jax.numpy as jnp
from jax import lax
import jax.experimental.pallas as pl
import jax.experimental.pallas.tpu as pltpu

S, D = 2048, 1024
HQ, HKV, DH = 32, 4, 128
SK = 2048
W = 512
REP = HQ // HKV
F = 3584
EPS = 1e-5
QSCALE = DH ** -0.5 * 1.4426950408889634
BM = 256
NB = S // BM
HM = BM // 2
NT = D // 128
NF = F // 128
NMOD = 6 * NT
SUB = 16
KH = HQ * DH // 2
NH = NT // 2
HH = HQ // 2
QH = D // 2
QT = QH // 128
NP = REP // 2
WB_WO, WB_AC, WB_V, WB_WQ = 0, 20, 30, 31
WB_SLOTS = 51
HC = {"m1": 0, "m2": 1, "m3": 2, "m4": 3, "m5": 4, "m6": 5, "m7": 6}
WC = {"m1": 0, "m3": 1, "m4": 2, "m6": 3, "m7": 4}
AC = {"m1": 0, "m2": 1, "m5": 2, "m6": 3, "m7": 4}

f32 = jnp.float32
bf16 = jnp.bfloat16
u32 = jnp.uint32
NT_DIMS = (((1,), (1,)), ((), ()))


def _rows(m8, n):
    return jnp.concatenate([m8] * (n // 8), axis=0) if n > 8 else m8


def _hint(x, m):
    return x if isinstance(x, int) else pl.multiple_of(x, m)


def _normalize(x):
    xc = x - jnp.mean(x, axis=-1, keepdims=True)
    return xc * lax.rsqrt(jnp.mean(xc * xc, axis=-1, keepdims=True) + EPS)


def _b(u):
    return pltpu.bitcast(u, bf16)


def _kernel(x_hbm, k_hbm, v_hbm, wq_hbm, wo_hbm, wr_hbm, wg_hbm, wu_hbm, wd_hbm, c_hbm, wmod_hbm,
            out_hbm,
            xo_v, k_v, ws_v, wr_v, wg_v, wu_v, wd_v, c_v, wmod_v,
            hce_v, hco_v, o_v, qa_v, qb_v, mod_v, wb_v, acca_v, accb_v, slab_v,
            sx, swq, swm, sw, so, sk, sm):
    x_v = xo_v.at[0]
    h2_v = xo_v.at[1]
    out_v = xo_v.at[2]
    k_u = k_v.bitcast(u32)
    ws_u = ws_v.bitcast(u32)
    wg_u = wg_v.bitcast(u32)
    wu_u = wu_v.bitcast(u32)
    wd_u = wd_v.bitcast(u32)
    wmod_u = wmod_v.bitcast(u32)
    hce_u = hce_v.bitcast(u32)
    hco_u = hco_v.bitcast(u32)
    o_u = o_v.bitcast(u32)
    qa_u = qa_v.bitcast(u32)
    qb_u = qb_v.bitcast(u32)
    wb_u = wb_v.bitcast(u32)

    cp_c = pltpu.make_async_copy(c_hbm, c_v, sm.at[0])
    cp_wr = pltpu.make_async_copy(wr_hbm, wr_v, sm.at[1])
    win = pl.ds(SK - W, W)
    cp_k = [pltpu.make_async_copy(k_hbm.at[g, win, :], k_v.at[g], sk.at[min(g, 1)])
            for g in range(HKV)]
    cp_v = [pltpu.make_async_copy(v_hbm.at[g, win, :], wb_v.at[WB_V, pl.ds(g * W, W), :], sk.at[1])
            for g in range(HKV)]
    cp_ve = pltpu.make_async_copy(v_hbm.at[0, win, :], hce_v.at[7 * QT], sk.at[0])
    cp_vo = pltpu.make_async_copy(v_hbm.at[0, win, :], hco_v.at[7 * QT], sk.at[0])

    def cp_x(i, sem=None):
        r = pl.ds(pl.multiple_of(i * BM, BM), BM)
        return pltpu.make_async_copy(x_hbm.at[r, :], x_v.at[r, :], sx.at[sem if sem is not None else i])

    def cp_out(i):
        r = pl.ds(pl.multiple_of(i * BM, BM), BM)
        return pltpu.make_async_copy(out_v.at[r, :], out_hbm.at[r, :], so.at[0])

    def cp_tile(w_hbm, w_v, sem, sem_of, n):
        return pltpu.make_async_copy(w_hbm.at[:, pl.ds(n * 128, 128)], w_v.at[n], sem.at[sem_of(n)])

    def cp_wq(n):
        return pltpu.make_async_copy(wq_hbm.at[:, pl.ds(n * 128, 128)], ws_v.at[n // 4, pl.ds((n % 4) * D, D), :],
                                     swq.at[n % NP if n < REP else NP + (n >= 2 * REP)])

    def cp_wo(n):
        return pltpu.make_async_copy(wo_hbm.at[:, pl.ds(n * 128, 128)], ws_v.at[NT + n], sw.at[0])

    def cp_wm(n):
        sem = min(n, 2 * NT) if isinstance(n, int) else n
        return pltpu.make_async_copy(wmod_hbm.at[:, pl.ds(_hint(n * 128, 128), 128)], wmod_v.at[n], swm.at[sem])

    cp_wg = functools.partial(cp_tile, wg_hbm, wg_v, sw, lambda n: 1)
    cp_wu = functools.partial(cp_tile, wu_hbm, wu_v, sw, lambda n: 2)
    cp_wd = functools.partial(cp_tile, wd_hbm, wd_v, sw, lambda n: 3)

    cp_c.start()
    cp_x(0).start()
    cp_x(1).start()
    cp_c.wait()
    for n in range(2 * NT):
        cp_wm(n).start()
    cc = c_v[...].astype(f32)
    sc16 = jnp.broadcast_to((cc * jax.nn.sigmoid(cc)).astype(bf16), (16, D))

    def mod_tile(n):
        r = jnp.dot(sc16, _b(wmod_u[n]), preferred_element_type=f32)[0:8]
        r = r.astype(bf16).astype(f32)
        if isinstance(n, int):
            r = 1.0 + r if n // NT == 4 else r
        else:
            r = (r + jnp.where(n >= NT, 1.0, 0.0)) * QSCALE
        mod_v[n] = r

    def mod(k, cols=None):
        if cols is not None:
            return mod_v[k * NT + cols]
        return jnp.concatenate([mod_v[k * NT + t] for t in range(NT)], axis=1)

    def store_hc(h, hc_v, r):
        ht, hb = h[:16], h[16:]
        a11, a12, a21, a22 = ht[:, :QH], ht[:, QH:], hb[:, :QH], hb[:, QH:]
        combos = (a11 + a22, a21 + a22, a11, a22, a11 + a12, a21 - a11, a12 - a22)
        for ci, val in enumerate(combos):
            vb = val.astype(bf16)
            for kt in range(QT):
                hc_v[ci * QT + kt, r, :] = vb[:, kt * 128:(kt + 1) * 128]

    def piece_rows(i, c):
        return (pl.ds(pl.multiple_of(i * BM + 16 * c, 16), 16),
                pl.ds(pl.multiple_of(i * BM + HM + 16 * c, 16), 16))

    def ln1_piece(i, hc_v, c):
        rt, rb = piece_rows(i, c)
        x = jnp.concatenate([x_v[rt, :], x_v[rb, :]], axis=0).astype(f32)
        h = _normalize(x) * _rows(mod(1), 32) + _rows(mod(0), 32)
        store_hc(h, hc_v, pl.ds(pl.multiple_of((i // 2) * HM + 16 * c, 16), 16))

    def normalize_block(i, dst):
        def piece(c, _):
            rt, rb = piece_rows(i, c)
            x = jnp.concatenate([x_v[rt, :], x_v[rb, :]], axis=0).astype(f32)
            dst[pl.ds(pl.multiple_of(32 * c, 32), 32), :] = _normalize(x)
            return 0

        lax.fori_loop(0, HM // 16, piece, 0)

    def modulate_block(src, hc_v):
        for c in range(HM // 16):
            h = src[32 * c:32 * c + 32, :] * _rows(mod(1), 32) + _rows(mod(0), 32)
            store_hc(h, hc_v, pl.ds(16 * c, 16))

    cp_x(0).wait()
    normalize_block(0, acca_v)
    cp_x(1).wait()
    normalize_block(1, accb_v)
    wq_first = [j + NP * hi for j in range(NP) for hi in range(2)]

    def first_vectors(n, _):
        cp_wm(n).wait()

        @pl.when(n == 11)
        def _():
            for nn in wq_first:
                cp_wq(nn).start()
            cp_k[0].start()
            cp_ve.start()
            cp_vo.start()

        mod_tile(n)
        return 0

    lax.fori_loop(0, 2 * NT, first_vectors, 0)

    def combo(job):
        if isinstance(job, int):
            pick = lambda a, b: a if job < 128 else b
            hint = lambda x, m: x
        else:
            is_q = job < 128
            pick = lambda a, b: jnp.where(is_q, a, b)
            hint = pl.multiple_of
        pair, grp_o = job // 8, job - 128
        lo = (pair // NP) * REP + pair % NP
        n = grp_o // 32
        r0 = hint(pick(job % 8, grp_o % 32) * 32, 32)
        half = pick(QH // 2, KH // 2)
        s1, base1 = pick(lo // 4, NT + n), pick((lo % 4) * (D // 2), 0)
        s2, base2 = pick((lo + NP) // 4, NT + NH + n), pick(((lo + NP) % 4) * (D // 2), 0)
        for k in range(4):
            r1 = hint(base1 + r0 + 8 * k, 8)
            r2 = hint(base2 + r0 + 8 * k, 8)
            b11 = _b(ws_u[s1, pl.ds(r1, 8), :]).astype(f32)
            b21 = _b(ws_u[s1, pl.ds(hint(r1 + half, 8), 8), :]).astype(f32)
            b12 = _b(ws_u[s2, pl.ds(r2, 8), :]).astype(f32)
            b22 = _b(ws_u[s2, pl.ds(hint(r2 + half, 8), 8), :]).astype(f32)
            for ci, val in enumerate((b11 + b22, b12 - b22, b21 - b11, b11 + b12, b21 + b22)):
                t = pair * 5 + ci
                slot = pick(WB_WQ + t // 4, WB_WO + ci * NH + n)
                row = hint(pick((t % 4) * QH, 0) + 2 * r0 + 16 * k, 16)
                wb_v[slot, pl.ds(row, 16), :] = val.astype(bf16)

    GQ = NP * 8

    def qprod(name, g, i, hc_u, jp):
        r = pl.ds(pl.multiple_of((i // 2) * (HM // 2), HM // 2), HM // 2)
        a = jnp.concatenate([_b(hc_u[HC[name] * QT + kt, r, :]) for kt in range(QT)], axis=1)
        if name == "m2":
            b = ws_u[2 * g, jp * (D // 2):jp * (D // 2) + QH // 2, :]
        elif name == "m5":
            b = ws_u[2 * g + 1, jp * (D // 2) + QH // 2:(jp + 1) * (D // 2), :]
        else:
            t = (g * NP + jp) * 5 + WC[name]
            b = wb_u[WB_WQ + t // 4, pl.ds(_hint((t % 4) * (QH // 2), QH // 2), QH // 2), :]
        return jnp.dot(a, _b(b), preferred_element_type=f32)

    def qstore(q_dst, j, half, val):
        q_dst[j, half * HM:(half + 1) * HM, :] = val.astype(bf16)

    def qproj_part(g, i, hc_u, q_dst, jp, part, carry):
        prod = lambda name: qprod(name, g, i, hc_u, jp)
        if part == 0:
            c22 = prod("m6")
            m3 = prod("m3")
            c22 = c22 + m3
            m5 = prod("m5")
            qstore(q_dst, jp + NP, 0, m3 + m5)
            return prod("m7") - m5, c22
        c11, c22 = carry
        m1 = prod("m1")
        c11 = c11 + m1
        c22 = c22 + m1
        m4 = prod("m4")
        qstore(q_dst, jp, 0, c11 + m4)
        m2 = prod("m2")
        qstore(q_dst, jp, 1, m4 + m2)
        qstore(q_dst, jp + NP, 1, c22 - m2)
        return None

    def kv_rows(g):
        return pl.ds(pl.multiple_of(g * (W // 2), W // 2), W // 2)

    def qk(g, q_src, j):
        return lax.dot_general(_b(q_src[j]), _b(k_u[g]), NT_DIMS, preferred_element_type=f32)

    def softmax_pv(g, i, j, s, v_src):
        m = jnp.max(s, axis=-1, keepdims=True)
        e = jnp.exp2(s - m)
        l = jnp.sum(e, axis=-1, keepdims=True)
        inv = pl.reciprocal(l, approx=True)
        inv = inv * (2.0 - l * inv)
        p = (e * inv).astype(bf16)
        o = jnp.dot(p, _b(v_src(g)), preferred_element_type=f32)
        o_v[g * REP + j, pl.ds(pl.multiple_of(i * BM, BM), BM), :] = o.astype(bf16)

    v_wb = lambda g: wb_u[WB_V, kv_rows(g), :]
    v_he = lambda g: hce_u[7 * QT]
    v_ho = lambda g: hco_u[7 * QT]

    def step(ga, ia, q_src, v_src, gq=None, iq=None, hc_u=None, q_dst=None, before=None, after=None):
        s = qk(ga, q_src, 0)
        carry = None
        for j in range(REP):
            s_next = qk(ga, q_src, j + 1) if j + 1 < REP else None
            if q_dst is not None:
                carry = qproj_part(gq, iq, hc_u, q_dst, j // 2, j % 2, carry)
            if before is not None:
                before(j)
            softmax_pv(ga, ia, j, s, v_src)
            if after is not None:
                after(j)
            s = s_next

    modulate_block(acca_v, hce_v)
    modulate_block(accb_v, hco_v)
    for jp in range(NP):
        cp_wq(jp).wait()
        cp_wq(jp + NP).wait()
        if jp == 1:
            cp_x(2, 2).start()
            cp_x(3, 2).start()
        for grp in range(jp * 8, (jp + 1) * 8):
            combo(grp)
        carry = qproj_part(0, 0, hce_u, qa_v, jp, 0, None)
        qproj_part(0, 0, hce_u, qa_v, jp, 1, carry)
    for i in range(4, NB):
        cp_x(i, 1 + i // 2).start()
    for n in range(REP, 2 * REP):
        cp_wq(n).start()
    for g in range(1, HKV):
        cp_k[g].start()
    for g in range(HKV):
        cp_v[g].start()
    cp_k[0].wait()
    cp_ve.wait()
    cp_vo.wait()

    def loop1(p, _):
        @pl.when(p == 1)
        def _():
            for n in range(REP, 2 * REP):
                cp_wq(n).wait()
            for n in range(2 * REP, 4 * REP):
                cp_wq(n).start()

        @pl.when(p == 2)
        def _():
            for n in range(NT):
                cp_wo(n).start()
            cp_wr.start()

        @pl.when(p == 3)
        def _():
            for n in range(2 * NT, NMOD):
                cp_wm(n).start()

        @pl.when(p < NB // 2 - 1)
        def _():
            cp_x(2 * p + 2, 2 + p).wait()
            cp_x(2 * p + 3, 2 + p).wait()

        @pl.when(p == 2)
        def _():
            for grp in range(GQ, 2 * GQ):
                combo(grp)

        t = 2 * p
        t2 = t + 2
        ia, ib = jnp.minimum(t + 2, NB - 2), jnp.minimum(t + 3, NB - 1)
        step(0, t, qa_u, v_he, 0, t + 1, hco_u, qb_v, after=lambda j: ln1_piece(ia, hce_v, j))
        step(0, t + 1, qb_u, v_ho, t2 // NB, t2 % NB, hce_u, qa_v, after=lambda j: ln1_piece(ib, hco_v, j))
        return 0

    lax.fori_loop(0, NB // 2, loop1, 0)

    for n in range(2 * REP, 4 * REP):
        cp_wq(n).wait()
    for g in range(1, HKV):
        cp_k[g].wait()
    for g in range(HKV):
        cp_v[g].wait()
    for n in range(NT):
        cp_wo(n).wait()

    NSTEP = HKV * NB

    def loop2(p, _):
        @pl.when(p == 0)
        def _():
            for n in range(NF):
                cp_wg(n).start()

        @pl.when(p == 1)
        def _():
            for n in range(NF):
                cp_wu(n).start()

        @pl.when(p == 2)
        def _():
            for n in range(NT):
                cp_wd(n).start()

        t = NB + 2 * p
        t1, t2 = t + 1, t + 2
        job = 2 * GQ + p * 2 * REP
        step(t // NB, t % NB, qa_u, v_wb, t1 // NB, t1 % NB, hco_u, qb_v, after=lambda j: combo(job + j))
        step(t1 // NB, t1 % NB, qb_u, v_wb, t2 // NB, t2 % NB, hce_u, qa_v, after=lambda j: combo(job + REP + j))
        return 0

    NC = (NSTEP - NB) // 2 - 1
    lax.fori_loop(0, NC, loop2, 0)
    JOBS_DONE = 2 * GQ + NC * 2 * REP

    ac_jobs = [(hd, rg) for hd in range(HH) for rg in range(HM // 16)]

    def a_combo(i, slot, jobs):
        for hd, rg in jobs:
            rt = pl.ds(pl.multiple_of(i * HM + rg * 8, 8), 8)
            rb = pl.ds(pl.multiple_of(i * HM + HM // 2 + rg * 8, 8), 8)
            a11 = _b(o_u[hd, rt, :]).astype(f32)
            a12 = _b(o_u[HH + hd, rt, :]).astype(f32)
            a21 = _b(o_u[hd, rb, :]).astype(f32)
            a22 = _b(o_u[HH + hd, rb, :]).astype(f32)
            r = hd * HM + rg * 16
            for ci, val in enumerate((a11 + a22, a21 + a22, a11 + a12, a21 - a11, a12 - a22)):
                wb_v[WB_AC + slot * 5 + ci, r:r + 16, :] = val.astype(bf16)

    cp_wr.wait()
    wr16 = jnp.broadcast_to(wr_v[...].reshape(1, D), (16, D))

    def olhs(kind, i, slot):
        if kind == "m3":
            r = pl.ds(pl.multiple_of(i * HM, HM // 2), HM // 2)
            return jnp.concatenate([_b(o_u[hd, r, :]) for hd in range(HH)], axis=1)
        if kind == "m4":
            r = pl.ds(pl.multiple_of(i * HM + HM // 2, HM // 2), HM // 2)
            return jnp.concatenate([_b(o_u[HH + hd, r, :]) for hd in range(HH)], axis=1)
        return jnp.concatenate(
            [_b(wb_u[WB_AC + slot * 5 + AC[kind], hd * (HM // 2):(hd + 1) * (HM // 2), :]) for hd in range(HH)],
            axis=1)

    def orhs(kind, n):
        if kind == "m2":
            return _b(ws_u[NT + n, 0:KH // 2, :])
        if kind == "m5":
            return _b(ws_u[NT + NH + n, KH // 2:KH, :])
        return _b(wb_u[WB_WO + WC[kind] * NH + n])

    def oprod(kind, i, slot, n):
        return jnp.dot(olhs(kind, i, slot), orhs(kind, n), preferred_element_type=f32)

    def epilogue(i, acc_r, c0, nc, sub):
        hs = []
        for o in range(0, nc, sub):
            r = pl.ds(pl.multiple_of(i * BM + c0 + o, sub), sub)
            x1 = x_v[r, :].astype(f32) + _rows(mod(2), sub) * acc_r[c0 + o:c0 + o + sub, :]
            h2 = _normalize(x1) * _rows(mod(4), sub) + _rows(mod(3), sub)
            h2b = h2.astype(bf16)
            h2_v[r, :] = h2b
            out_v[r, :] = (x1 + _rows(mod(5), sub) * h2).astype(bf16)
            hs.append(h2b)
        h2b = jnp.concatenate(hs, axis=0) if len(hs) > 1 else hs[0]
        score = lax.dot_general(wr16, h2b, NT_DIMS, preferred_element_type=f32)
        return score[0:8, :].astype(bf16).astype(f32)

    def update_best(state, i, scores):
        best_v, best_i = state
        r = jnp.concatenate(scores, axis=1)
        rows = i * BM + lax.broadcasted_iota(jnp.int32, (8, BM), 1)
        better = r > best_v
        return jnp.where(better, r, best_v), jnp.where(better, rows, best_i)

    def block_steps(i, slot, acc_w, i_prev, acc_r, result, inext=None, snext=None, do_epi=True):
        scores = []
        nprod = NH * 7
        per = len(ac_jobs) // nprod
        extra = len(ac_jobs) - per * nprod
        pos = [0, 0]

        def fill():
            cnt = per + (1 if pos[1] < extra else 0)
            if inext is not None:
                a_combo(inext, snext, ac_jobs[pos[0]:pos[0] + cnt])
            pos[0] += cnt
            pos[1] += 1

        def prod(kind, n):
            val = oprod(kind, i, slot, n)
            fill()
            return val

        for n in range(NH):
            cl = slice(n * 128, (n + 1) * 128)
            cr = slice((NH + n) * 128, (NH + n + 1) * 128)
            c22 = prod("m6", n)
            yield
            m3 = prod("m3", n)
            yield
            c22 = c22 + m3
            m5 = prod("m5", n)
            yield
            acc_w[0:HM, cr] = m3 + m5
            c11 = prod("m7", n) - m5
            yield
            m1 = prod("m1", n)
            yield
            c11 = c11 + m1
            c22 = c22 + m1
            m4 = prod("m4", n)
            yield
            acc_w[0:HM, cl] = c11 + m4
            m2 = prod("m2", n)
            acc_w[HM:BM, cl] = m4 + m2
            acc_w[HM:BM, cr] = c22 - m2
            if do_epi and n in (1, 3):
                scores.append(epilogue(i_prev, acc_r, (n // 2) * HM, HM, SUB))
            if n < NH - 1:
                yield
        if do_epi:
            result[0] = update_best(result[0], i_prev, scores)
            cp_out(i_prev).start()

    def block(i, slot, acc_w, i_prev, acc_r, state, inext=None, snext=None):
        result = [state]
        for _ in block_steps(i, slot, acc_w, i_prev, acc_r, result, inext, snext):
            pass
        return result[0]

    for n in range(2 * NT, NMOD):
        cp_wm(n).wait()
    step(HKV - 1, NB - 2, qa_u, v_wb, HKV - 1, NB - 1, hco_u, qb_v,
         after=lambda j: (combo(JOBS_DONE + 2 * j), combo(JOBS_DONE + 2 * j + 1),
                          a_combo(0, 0, ac_jobs[j * 16:(j + 1) * 16])))

    first = block_steps(0, 0, acca_v, None, None, None, 1, 1, do_epi=False)

    def first_fill(j):
        for n in range(2 * NT + 4 * j, 2 * NT + 4 * j + 4):
            mod_tile(n)
        for _ in range(4 if j % 2 else 3):
            next(first, None)

    step(HKV - 1, NB - 1, qb_u, v_wb, before=first_fill)
    for _ in first:
        pass

    state = (jnp.full((8, BM), -jnp.inf, f32), jnp.zeros((8, BM), jnp.int32))

    def loopb(p, state):
        i = 2 * p
        state = block(i + 1, 1, accb_v, i, acca_v, state, i + 2, 0)
        state = block(i + 2, 0, acca_v, i + 1, accb_v, state, i + 3, 1)
        return state

    state = lax.fori_loop(0, NB // 2 - 1, loopb, state)
    for n in range(NF):
        cp_wg(n).wait()
        cp_wu(n).wait()
    for n in range(NT):
        cp_wd(n).wait()
    state = block(NB - 1, 1, accb_v, NB - 2, acca_v, state)
    scores = [epilogue(NB - 1, accb_v, c * 128, 128, 64) for c in range(BM // 128)]
    best_v, best_i = update_best(state, NB - 1, scores)
    cp_out(NB - 1).start()

    rmax = jnp.max(best_v, axis=1, keepdims=True)
    idx = jnp.min(jnp.where(best_v == rmax, best_i, S), axis=1, keepdims=True)
    base = pl.multiple_of((idx[0, 0] // 16) * 16, 16)
    hs = h2_v[pl.ds(base, 16), :]
    acts = []
    for n in range(NF):
        gate = jnp.dot(hs, _b(wg_u[n]), preferred_element_type=f32).astype(bf16).astype(f32)
        up = jnp.dot(hs, _b(wu_u[n]), preferred_element_type=f32).astype(bf16).astype(f32)
        acts.append(((gate * jax.nn.sigmoid(gate)).astype(bf16).astype(f32) * up).astype(bf16))
    act = jnp.concatenate(acts, axis=1)
    old = out_v[pl.ds(base, 16), :].astype(f32)
    sel = base + lax.broadcasted_iota(jnp.int32, (16, 1), 0) == idx[0:1, :]
    weight = jax.nn.sigmoid(rmax[0:1, :])
    for n in range(NT):
        cols = slice(n * 128, (n + 1) * 128)
        y = jnp.dot(act, _b(wd_u[n]), preferred_element_type=f32).astype(bf16).astype(f32)
        new = old[:, cols] + _rows(mod(5, n), 16) * (y * weight)
        slab_v[:, cols] = jnp.where(sel, new, old[:, cols]).astype(bf16)
    for i in range(NB):
        cp_out(i).wait()
    cp_slab = pltpu.make_async_copy(slab_v, out_hbm.at[pl.ds(base, 16), :], sm.at[2])
    cp_slab.start()
    cp_slab.wait()


@jax.jit
def pallas_adaLN_cond__sliding_block_cached__moe_arch_mod__prompt_kernel(
        A_x, A_k_cache, A_v_cache, A_wq, A_wo, B_x, B_w_r, B_w_gate, B_w_up, B_w_down, c, w_mod):
    x = A_x.reshape(S, D)
    k = A_k_cache.reshape(HKV, SK, DH)
    v = A_v_cache.reshape(HKV, SK, DH)
    wr = B_w_r
    anyspec = pl.BlockSpec(memory_space=pl.ANY)
    dma = pltpu.SemaphoreType.DMA
    out = pl.pallas_call(
        _kernel,
        out_shape=jax.ShapeDtypeStruct((S, D), bf16),
        in_specs=[anyspec] * 11,
        out_specs=anyspec,
        scratch_shapes=[
            pltpu.VMEM((3, S, D), bf16),
            pltpu.VMEM((HKV, W, DH), bf16),
            pltpu.VMEM((2 * NT, HQ * DH, 128), bf16),
            pltpu.VMEM((D,), bf16),
            pltpu.VMEM((NF, D, 128), bf16),
            pltpu.VMEM((NF, D, 128), bf16),
            pltpu.VMEM((NT, F, 128), bf16),
            pltpu.VMEM((1, D), bf16),
            pltpu.VMEM((NMOD, D, 128), bf16),
            pltpu.VMEM((7 * QT + 1, S // 4, 128), bf16),
            pltpu.VMEM((7 * QT + 1, S // 4, 128), bf16),
            pltpu.VMEM((HQ, S, 128), bf16),
            pltpu.VMEM((REP, BM, 128), bf16),
            pltpu.VMEM((REP, BM, 128), bf16),
            pltpu.VMEM((NMOD, 8, 128), f32),
            pltpu.VMEM((WB_SLOTS, KH, 128), bf16),
            pltpu.VMEM((BM, D), f32),
            pltpu.VMEM((BM, D), f32),
            pltpu.VMEM((16, D), bf16),
            dma((1 + NB // 2,)), dma((NP + 2,)), dma((2 * NT + 1,)), dma((4,)), dma((1,)), dma((2,)), dma((3,)),
        ],
        compiler_params=pltpu.CompilerParams(vmem_limit_bytes=124 * 1024 * 1024),
    )(x, k, v, A_wq, A_wo, wr, B_w_gate, B_w_up, B_w_down, c, w_mod)
    return out.reshape(1, S, D)
```
